```python
import jax
import jax.numpy as jnp

def _softmax(x, axis=-1):
    return jax.nn.softmax(x, axis=axis)
def _gelu(x):
    return jax.nn.gelu(x, approximate=True)
def _silu(x):
    return jax.nn.silu(x)
def _sigmoid(x):
    return jax.nn.sigmoid(x)
def _layernorm(x, axis=-1, eps=1e-5):
    m = jnp.mean(x, axis=axis, keepdims=True)
    v = jnp.var(x, axis=axis, keepdims=True)
    return (x - m) / jnp.sqrt(v + eps)
def _scatter_add(tgt, idx, src, axis=0):
    return tgt.at[idx].add(src)
def _segment_sum(src, seg, n):
    return jax.ops.segment_sum(src, seg, n)
class _Rng:
    def __init__(self, key):
        self._k = key
    def _next(self):
        self._k, sub = jax.random.split(self._k)
        return sub
    def normal(self, shape):
        return jax.random.normal(self._next(), shape, dtype=jnp.bfloat16)
    def randint(self, lo, hi, shape):
        return jax.random.randint(self._next(), shape, lo, hi, dtype=jnp.int32)
    def uniform(self, shape, lo=0.0, hi=1.0):
        return jax.random.uniform(self._next(), shape, jnp.bfloat16, lo, hi)
    def permutation(self, n):
        return jax.random.permutation(self._next(), n)


kernel_name = 'recurrent_scan__sliding_block_cached__moe_arch_mod__decode'

def setup_inputs():
    _rng = _Rng(jax.random.key(int.from_bytes(__import__("os").urandom(4), "little")))
    _w = (lambda a: (lambda t: t.astype(jnp.bfloat16) if jnp.issubdtype(t.dtype, jnp.floating) else t)(jnp.asarray(a)))
    def _A_setup():
        B, Sq, D = 1, 1, 512
        Hq, Hkv, Sk, Dh = 32, 32, 32768, 128
        assert Hq % Hkv == 0, (Hq, Hkv)
        return {
            "x": _w((lambda *s: _rng.normal(s) * 0.05)(B, Sq, D)),
            "k_cache": _w((lambda *s: _rng.normal(s) * 0.05)(B, Hkv, Sk, Dh)),
            "v_cache": _w((lambda *s: _rng.normal(s) * 0.05)(B, Hkv, Sk, Dh)),
            "wq": _w((lambda *s: _rng.normal(s) * 0.05)(D, Hq * Dh) * (D ** -0.5)),
            "wo": _w((lambda *s: _rng.normal(s) * 0.05)(Hq * Dh, D) * ((Hq * Dh) ** -0.5)),
        }
    _A_in = _A_setup()

    def _B_setup():
        B, S, D, F, C = 1, 1, 512, 1376, 1
        return {
            "x": _w((lambda *s: _rng.normal(s) * 0.05)(B, S, D)),
            "w_r": _w((lambda *s: _rng.normal(s) * 0.05)(D)),
            "w_gate": _w((lambda *s: _rng.normal(s) * 0.05)(D, F)),
            "w_up": _w((lambda *s: _rng.normal(s) * 0.05)(D, F)),
            "w_down": _w((lambda *s: _rng.normal(s) * 0.05)(F, D)),
        }
    _B_in = _B_setup()

    return {
        "A_x": _A_in["x"],
        "A_k_cache": _A_in["k_cache"],
        "A_v_cache": _A_in["v_cache"],
        "A_wq": _A_in["wq"],
        "A_wo": _A_in["wo"],
        "B_x": _B_in["x"],
        "B_w_r": _B_in["w_r"],
        "B_w_gate": _B_in["w_gate"],
        "B_w_up": _B_in["w_up"],
        "B_w_down": _B_in["w_down"],
    }

def reference(A_x, A_k_cache, A_v_cache, A_wq, A_wo, B_x, B_w_r, B_w_gate, B_w_up, B_w_down):
    def _A_ref(x, k_cache, v_cache, wq, wo):
        B, Sq, D = x.shape
        Hq, Dh = 32, 128
        Hkv, Sk = k_cache.shape[1], k_cache.shape[2]
        W = min(4096, max(256, Sk // 4))
        rep = Hq // Hkv
        q = (lambda x, *d: x.transpose(*d))((x @ wq).reshape(B, Sq, Hq, Dh), 0, 2, 1, 3)
        k = jnp.repeat(k_cache[:, :, Sk - W:, :], rep, axis=1)
        v = jnp.repeat(v_cache[:, :, Sk - W:, :], rep, axis=1)
        scores = jnp.einsum("bhqd,bhkd->bhqk", q, k) * (Dh ** -0.5)
        p = _softmax(scores, axis=-1)
        o = jnp.einsum("bhqk,bhkd->bhqd", p, v)
        return (lambda x, *d: x.transpose(*d))(o, 0, 2, 1, 3).reshape(B, Sq, Hq * Dh) @ wo

    def _B_ref(x, w_r, w_gate, w_up, w_down):
        B, S, D = x.shape
        C = 1
        r = x @ w_r
        idx = jnp.argsort(-r, axis=-1)[:, :C]
        idx_e = jnp.repeat(idx.reshape(B, C, 1), D, axis=2)
        x_sel = jnp.take_along_axis(x, idx_e, axis=1)
        g = _silu(x_sel @ w_gate)
        u = x_sel @ w_up
        y = (g * u) @ w_down
        r_sel = _sigmoid(jnp.take_along_axis(r, idx, axis=1))
        y = y * r_sel.reshape(B, C, 1)
        b_off = (jnp.arange(B) * S).reshape(B, 1)
        flat_idx = (idx + b_off).reshape(B * C)
        zero = (x * 0.0).reshape(B * S, D)
        upd = _scatter_add(zero, flat_idx, y.reshape(B * C, D), axis=0)
        return x + upd.reshape(B, S, D)

    x = A_x
    xn = _layernorm(x, axis=-1)
    s = _A_ref(xn, A_k_cache, A_v_cache, A_wq, A_wo)
    g = _silu(_B_ref(xn, B_w_r, B_w_gate, B_w_up, B_w_down))
    return x + s * g
```

```python
import jax
import jax.numpy as jnp
import jax.experimental.pallas as pl
import jax.experimental.pallas.tpu as pltpu

D = 512; NH = 32; DH = 128; SK = 32768; W = 4096; F = 1376
BF16 = jnp.bfloat16; F32 = jnp.float32
_NT = (((1,), (1,)), ((), ()))
LONG, SHORT = 1, 0


def build(name='k3', A0=64, Q0=1024, WO0=16, T=88, TP=93, TA=(1, 1), TQP=10, TM=46, TE=28, TC=1, FP=2, TF=(1, 1), TW=40, TG=(1, 1), FH=9, WL=53, WP=5,
          EG=(0, 4, 8, 16, 24, 32), nbc=True, NA=14, T0=None, TN=(40, 1, 20), only=None, bc=False, last=16, scopes=False, cm=1, IL=0):
    PR = 256
    TP = TP or T
    WR = 64; NB = 8; BR = NH * DH // NB
    FC = 128; NF = -(-F // FC)
    QS = 4; KS = W // QS; N0 = 18
    FB = -(-F // BR)
    import contextlib
    sc = (lambda n: jax.named_scope(n)) if scopes else (lambda n: contextlib.nullcontext())
    on = lambda s: only is None or s in only

    def kernel(x_h, k_h, v_h, wq_h, wo_h, wr_h, wg_h, wu_h, wd_h, out_ref,
               x_v, wr_v, wq_v, kv_v, w_v, q_v, s_v, p_v, l_v, c_v,
               s_x, s_wq, s_f, s_kv, s_e, s_wo):
        kv_h = (k_h, v_h)
        mul = lambda a, m: a if isinstance(a, int) else pl.multiple_of(a, m)

        def load(ref, lead, ro, n, cols=slice(None)):
            if not bc:
                return ref[lead + (pl.ds(mul(ro, 16), n), cols)]
            return pltpu.bitcast(ref.bitcast(jnp.uint32)[lead + (pl.ds(mul(ro // 2, 8), n // 2), cols)], BF16)

        def piece(t, u, c):
            n = (u & 1) * NA + c
            h = (u & ~1) + (n & 1)
            j = n >> 1
            ro = A0 + ((j >> 1) + (j & 1) * ((NA + 1) // 2)) * PR
            pltpu.make_async_copy(kv_h[t].at[0, h, pl.ds(mul(SK - W + ro, 16), PR), :], kv_v.at[t, h, pl.ds(mul(ro, 16), PR), :],
                                  s_kv.at[t, (u >> 1) & 1]).start(priority=SHORT)

        def wait_pair(t, p):
            r_ = kv_v.at[t, pl.ds(2 * p, 2), pl.ds(A0, NA * PR), :]
            pltpu.make_async_copy(r_, r_, s_kv.at[t, p & 1]).wait()

        def wo_rows(ro, n, s):
            return pltpu.make_async_copy(wo_h.at[pl.ds(ro, n), :], w_v.at[pl.ds(ro, n), :], s)

        def wo_row(n):
            return (n & 7) * BR + WO0 + (n >> 3) * WR

        def wo_copy(n):
            return wo_rows(mul(wo_row(n), 16), WR, s_wo.at[n])

        def wo_half(u):
            n = u - jnp.where(u >= N0, N0, 0)
            wo_rows(mul(wo_row(n) + jnp.where(u >= N0, WR // 2, 0), 16), WR // 2, s_wo.at[n]).start(priority=SHORT)

        def column(h, o):
            o = jnp.concatenate([o.astype(BF16).astype(F32)] * (DH // 8), axis=0)
            dg = jnp.where(jax.lax.broadcasted_iota(jnp.int32, (DH, DH), 0) == jax.lax.broadcasted_iota(jnp.int32, (DH, DH), 1), o, 0.0)
            c_v[pl.ds(mul(h * DH, DH), DH), :] = jnp.broadcast_to(jnp.sum(dg, axis=-1, keepdims=True), (DH, DH))

        def wq_piece(n):
            g = (n >> 3) + (n & 7) * 8
            for r_, c0, c1 in ((g, Q0, NH * DH), ((g + 1) & 63, 0, Q0)):
                if c1 > c0:
                    ro = mul(r_ * 8, 8)
                    pltpu.make_async_copy(wq_h.at[pl.ds(ro, 8), pl.ds(c0, c1 - c0)], wq_v.at[pl.ds(ro, 8), pl.ds(c0, c1 - c0)], s_wq).start(priority=SHORT)

        copy_x = pltpu.make_async_copy(x_h, x_v, s_x.at[0])
        copy_wr = pltpu.make_async_copy(wr_h, wr_v, s_x.at[1])
        long_e = [[pltpu.make_async_copy(kv_h[t].at[0, pl.ds(a, b - a), pl.ds(SK - W + ro, n), :], kv_v.at[t, pl.ds(a, b - a), pl.ds(ro, n), :], s_e.at[g])
                   for t in range(2) for ro, n in ((A0 + NA * PR, W - A0 - NA * PR), (0, A0)) if n] for g, (a, b) in enumerate(zip(EG, EG[1:]))]
        GO, UO, DO = NH * DH, NH * DH + F, NH * DH + 2 * F
        long_f = [[pltpu.make_async_copy(a.at[pl.ds(ro, n), :], w_v.at[pl.ds(b + ro, n), :], s_f.at[u]) for a, b in ((wg_h, GO), (wu_h, UO), (wd_h, DO))]
                  for u, (ro, n) in enumerate(((0, FH * FC), (FH * FC, F - FH * FC)))]
        long_wo = [wo_copy(56 + b) for b in range(NB - 1)] + [wo_rows(a, n, s_wo.at[63]) for a, n in ((wo_row(63), WR - WO0), (0, WO0)) if n]

        longs = sum(long_e + long_f, [])
        longs[0].start(priority=LONG)
        pl.delay(1)
        wq_piece(0)
        copy_x.start(priority=SHORT)
        copy_wr.start(priority=SHORT)
        pl.delay(T0 or TP - 40)
        n0 = 6
        per = -(-(len(longs) - 1) // (n0 - 1))
        for n in range(1, n0):
            wq_piece(n)
            for c in longs[1 + (n - 1) * per:1 + n * per]:
                pl.delay(1)
                c.start(priority=LONG)
            pl.delay(TP - 3 * per)
        wq_piece(n0)
        copy_x.wait()
        copy_wr.wait()
        x = x_v[0].astype(F32)
        mean = jnp.mean(x, axis=-1, keepdims=True)
        xc = x - mean
        pl.delay(TN[0])
        wq_piece(n0 + 1)
        var = jnp.mean(jnp.square(xc), axis=-1, keepdims=True)
        xn_b = (xc / jnp.sqrt(var + 1e-5)).astype(BF16)
        xn = xn_b.astype(F32)
        xn8 = jnp.broadcast_to(xn_b, (8, D))
        pl.delay(TN[1])
        wq_piece(n0 + 2)
        r = jnp.sum(xn * wr_v[...].reshape(1, D).astype(F32), axis=-1, keepdims=True)
        p_v[...] = jnp.zeros(p_v.shape, F32)
        l_v[...] = jnp.ones(l_v.shape, F32)
        pl.delay(TN[2])

        def pro1(n, c):
            wq_piece(n)
            pl.delay(TP)
            return c

        def pro2(c, carry):
            for t, b in ((0, 0), (0, 1), (1, 0)):
                piece(t, b, c)
                pl.delay(TP)
            return carry
        jax.lax.fori_loop(n0 + 3, 64, pro1, 0)
        with sc('pro2'):
            jax.lax.fori_loop(0, NA, pro2, 0)
        pltpu.make_async_copy(wq_v, wq_v, s_wq).wait()

        scale = DH ** -0.5

        def pv_slice(t, h, c, o, n):
            p = jnp.concatenate([p_v[c + u] for u in range(n)], axis=1).astype(BF16)
            return o + jnp.dot(p, load(kv_v, (t, h), c * (KS // 2), n * KS // 2), preferred_element_type=F32)

        def head(i, carry):
            def first(c):
                @pl.when(i < NH - 2)
                def _():
                    piece(0, i + 2, c)
                    pl.delay(T)

            def second(c, n):
                @pl.when(i < NH - 1)
                def _():
                    piece(1, i + 1, c)

                @pl.when(i == NH - 1)
                def _():
                    wo_copy(n).start(priority=SHORT)

            def idle(c, carry):
                first(c)
                piece(1, i + 1, c)
                pl.delay(T)
                return carry
            def third(c, n):
                @pl.when(i < NH - 2)
                def _():
                    piece(0, i + 2, c)

                @pl.when(i >= NH - 2)
                def _():
                    wo_copy(n).start(priority=SHORT)
            c0 = NA - QS * (1 + IL) - 3
            jax.lax.fori_loop(0, jnp.where(i < NH - 1, c0, 0), idle, 0)
            for g, a in enumerate(EG[:-1]):
                @pl.when(i == a)
                def _():
                    for c in long_e[g]:
                        c.wait()
                    if g == len(EG) - 2:
                        for c in long_wo:
                            c.start(priority=LONG)
                            pl.delay(1)
            wait_pair(i & 1, i >> 1)
            hp = jnp.maximum(i - 1, 0)
            tp = jnp.minimum(i, 1)
            nf = lambda u: jnp.where(i == NH - 2, u, 6 + 2 * u)

            third(c0, nf(0))
            pl.delay(TQP if on('p') else T)
            o = jnp.zeros((8, DH), F32)
            if on('p'):
                l_v[...] = jnp.broadcast_to(jnp.sum(l_v[...], axis=-1, keepdims=True), (8, DH))
                q_v[...] = jnp.dot(xn8, load(wq_v, (), 0, D, pl.ds(pl.multiple_of(i * DH, DH), DH)), preferred_element_type=F32)
                o = pv_slice(tp, hp, 4, o, 2)
            second(c0, 7)
            pl.delay(1 if on('p') else T)

            def att(c, carry):
                mx, o = carry
                third(c0 + 1 + c, nf(1 + c))
                pl.delay(TA[0] if on('a') else T)
                if on('a'):
                    s = jax.lax.dot_general(q_v[...].astype(BF16), load(kv_v, (0, i), c * KS, KS), _NT, preferred_element_type=F32) * scale
                    o = pv_slice(tp, hp, c, o, 1)
                second(c0 + 1 + c, 9 + 2 * c)
                if on('a'):
                    s_v[c] = s
                    for u in range(KS // DH):
                        mx = jnp.maximum(mx, s[:, u * DH:(u + 1) * DH])
                pl.delay(TA[1] if on('a') else T)
                if IL:
                    @pl.when(i < NH - 1)
                    def _():
                        idle(c0 + 1 + QS + c, 0)
                return mx, o
            mx, o = jax.lax.fori_loop(0, QS, att, (jnp.full((8, DH), -jnp.inf, F32), o))

            third(NA - 2, nf(5))
            pl.delay(TM if on('m') else T)
            if on('m'):
                q_v[...] = jnp.broadcast_to(jnp.max(mx, axis=-1, keepdims=True), (8, DH))
                o = pv_slice(tp, hp, 6, o, 2)
                o = o / l_v[...]
            second(NA - 2, 17)
            pl.delay(1 if on('m') else T)

            @pl.when(i < NH - 2)
            def _():
                piece(0, i + 2, NA - 1)
            if on('c'):
                column(hp, o)
            pl.delay(TC if on('c') else T)

            @pl.when(i < NH - 1)
            def _():
                piece(1, i + 1, NA - 1)
                pl.delay(TE if on('e') else T)
            if on('e'):
                tot = jnp.zeros((8, DH), F32)
                m = jnp.concatenate([q_v[...]] * (KS // DH), axis=1)
                for c in range(QS):
                    p = jnp.exp(s_v[c] - m)
                    p_v[2 * c] = p[:, :KS // 2]
                    p_v[2 * c + 1] = p[:, KS // 2:]
                    for u in range(KS // DH):
                        tot = tot + p[:, u * DH:(u + 1) * DH]
                l_v[...] = tot
            return carry
        with sc('loop'):
            jax.lax.fori_loop(0, NH, head, 0)

        with sc('fwait'):
            for c in long_f[0]:
                c.wait()

        def proj(ro, n, part):
            prod = load(w_v, (), ro, n).astype(F32) * jnp.concatenate([c_v[pl.ds(mul(ro, 8), n), :]] * (D // DH), axis=1)
            return part + prod.reshape(n // 8, 8, D).sum(axis=0)

        def one(n, part):
            wo_copy(n).wait()
            return proj(wo_row(n), WR, part)

        def ffn(j, carry):
            hid, y, o, part = carry
            f0 = jnp.minimum(j * FC, F - FC)
            fp = jnp.maximum((j - 1) * FC, 0)
            wo_copy(N0 + 2 * j).start(priority=SHORT)

            @pl.when(j == FH)
            def _():
                for c in long_f[1]:
                    c.wait()
            for u in range(FP):
                wo_copy(FP * j + u).wait()
            pl.delay(TF[0])
            gt = jax.lax.dot_general(xn8, load(w_v, (), GO + f0, FC), _NT, preferred_element_type=F32)
            up = jax.lax.dot_general(xn8, load(w_v, (), UO + f0, FC), _NT, preferred_element_type=F32)
            o = jnp.where(j < 2 * QS, pv_slice(1, NH - 1, jnp.minimum(j, 2 * QS - 1), o, 1), o)
            t = jnp.dot(hid.astype(BF16), load(w_v, (), DO + fp, FC), preferred_element_type=F32)
            wo_copy(N0 + 1 + 2 * j).start(priority=SHORT)
            for u in range(FP):
                part = proj(wo_row(FP * j + u), WR, part)
            col = f0 + jax.lax.broadcasted_iota(jnp.int32, (8, FC), 1)
            hid = jnp.where(col >= j * FC, jax.nn.silu(gt) * up, 0.0)
            y = jnp.where(j > 0, y + t, y)
            pl.delay(TF[1])
            return hid, y, o, part
        zd = jnp.zeros((8, D), F32)
        with sc('ffn'):
            hid, y, o, part = jax.lax.fori_loop(0, NF, ffn, (jnp.zeros((8, FC), F32), zd, jnp.zeros((8, DH), F32), zd))
        n1 = N0 + 2 * NF
        wo_copy(n1).start(priority=SHORT)
        q_v[...] = o / jnp.sum(l_v[...], axis=-1, keepdims=True)
        y = y + jnp.dot(hid.astype(BF16), load(w_v, (), DO + F - FC, FC), preferred_element_type=F32)
        pl.delay(TG[0])
        wo_copy(n1 + 1).start(priority=SHORT)
        column(NH - 1, q_v[...])
        gate = jax.nn.silu(xn + (xn * 0.0 + y * jax.nn.sigmoid(r)))
        pl.delay(TG[1])

        ns = 55 - n1 - 2

        def slot(c, part):
            wo_copy(n1 + 2 + c).start(priority=SHORT)
            part = one(FP * NF + 2 * c + 1, one(FP * NF + 2 * c, part))
            part = jax.lax.fori_loop(0, (c >= ns - WP).astype(jnp.int32), lambda u, t: one(56 + c - ns + WP, t), part)
            pl.delay(TW)
            return part
        with sc('proj'):
            part = jax.lax.fori_loop(0, ns, slot, part)
        a_ = wo_row(55)
        tail = [(a_, WR - last), (a_ + WR - last, last)] if last else [(a_, WR)]
        tc = [wo_rows(a, n, s_wo.at[(55, 64)[c]]) for c, (a, n) in enumerate(tail)]
        for c in tc:
            c.start(priority=SHORT)
            pl.delay(1)
        n2 = FP * NF + 2 * ns
        part = jax.lax.fori_loop(n2, WL + NB - 1 - WP, lambda n, t: one(jnp.where(n < WL, n, n - WL + 56 + WP), t), part)
        with sc('wwait'):
            for c in long_wo[NB - 1:]:
                c.wait()
        part = proj(NH * DH - WR + WO0, WR - WO0, proj(0, WO0, part) if WO0 else part)
        with sc('one'):
            part = jax.lax.fori_loop(WL, 55, one, part)
        for c, (a, n) in enumerate(tail):
            with sc(f't{c}'):
                tc[c].wait()
            part = proj(a, n, part)
        s_out = jnp.sum(part, axis=0, keepdims=True)
        res = jnp.broadcast_to(x, (8, D)) + jnp.broadcast_to(s_out, (8, D)) * gate
        out_ref[0] = res.astype(out_ref.dtype)[0:1]

    def fn(A_x, A_k_cache, A_v_cache, A_wq, A_wo, B_x, B_w_r, B_w_gate, B_w_up, B_w_down):
        hbm = pl.BlockSpec(memory_space=pltpu.HBM)
        dma = pltpu.SemaphoreType.DMA
        V = pltpu.VMEM
        return pl.pallas_call(
            kernel, name=name, out_shape=jax.ShapeDtypeStruct((1, 1, D), BF16), in_specs=[hbm] * 9,
            out_specs=pl.BlockSpec(memory_space=pltpu.VMEM),
            scratch_shapes=[V((1, 1, D), BF16), V((D,), BF16), V((D, NH * DH), BF16), V((2, NH, W, DH), BF16), V((NH * DH + 3 * F, D), BF16),
                            V((8, DH), F32), V((QS, 8, KS), F32), V((2 * QS, 8, KS // 2), F32), V((8, DH), F32), V((NH * DH, DH), F32),
                            dma((2,)), dma, dma((2,)), dma((2, 2)), dma((len(EG) - 1,)), dma((65,))],
            compiler_params=pltpu.CompilerParams(vmem_limit_bytes=100 * 1024 * 1024, disable_semaphore_checks=True, disable_bounds_checks=nbc),
        )(A_x, A_k_cache, A_v_cache, A_wq, A_wo, B_w_r, B_w_gate.T, B_w_up.T, B_w_down)
    return fn


pallas_recurrent_scan__sliding_block_cached__moe_arch_mod__decode_kernel = jax.jit(build(T=87,TP=90,TW=30))
```

```python
import jax
import jax.numpy as jnp
import jax.experimental.pallas as pl
import jax.experimental.pallas.tpu as pltpu

D = 512; NH = 32; DH = 128; SK = 32768; W = 4096; F = 1376
BF16 = jnp.bfloat16; F32 = jnp.float32
_NT = (((1,), (1,)), ((), ()))
LONG, SHORT = 1, 0


def build(name='k3', A0=(128, 64), Q0=2048, WO0=32, T=91, TP=None, TA=(1, 1), TQP=14, TM=24, TE=36, TC=1, FP=2, TF=(1, 1), TW=36, TG=(1, 1), FS=(0, 6, 8, 10), WL=53, WP=5,
          EG=(0, 2, 6, 12, 18, 24, 32), nbc=True, NA=15, T0=75, TN=(40, 1, 20), only=None, bc=False, last=16, scopes=False, cm=1, IL=0, es=0, DK=3, junk=0, KE=96, ev=2, TK=50):
    PR = 256
    NN = (NA - DK, NA)
    AA = (A0, A0) if isinstance(A0, int) else A0
    TI = (T,) if isinstance(T, int) else T
    SP = len(TI)
    T = sum(TI) + SP - 1
    TP = TP or T
    WR = 64; NB = 8; BR = NH * DH // NB
    FC = 128; NF = -(-F // FC)
    QS = 4; KS = W // QS; N0 = 18
    FB = -(-F // BR)
    import contextlib
    sc = (lambda n: jax.named_scope(n)) if scopes else (lambda n: contextlib.nullcontext())
    on = lambda s: only is None or s in only

    def kernel(x_h, k_h, v_h, wq_h, wo_h, wr_h, wg_h, wu_h, wd_h, out_ref,
               x_v, wr_v, wq_v, kv_v, w_v, q_v, s_v, p_v, l_v, c_v,
               s_x, s_wq, s_f, s_kv, s_e, s_wo):
        kv_h = (k_h, v_h)
        mul = lambda a, m: a if isinstance(a, int) else pl.multiple_of(a, m)

        def load(ref, lead, ro, n, cols=slice(None)):
            if not bc:
                return ref[lead + (pl.ds(mul(ro, 16), n), cols)]
            return pltpu.bitcast(ref.bitcast(jnp.uint32)[lead + (pl.ds(mul(ro // 2, 8), n // 2), cols)], BF16)

        def piece(t, u, c, d=0):
            n = (u & 1) * NN[t] + c - (NA - NN[t])
            h = (u & ~1) + (n & 1)
            j = n >> 1
            ro = AA[t] + ((j >> 1) + (j & 1) * ((NN[t] + 1) // 2)) * PR
            if d:
                for e in range(SP):
                    rows(t, h, ro + e * (PR // SP), PR // SP)
                    pl.delay(d[e])
            else:
                rows(t, h, ro, PR)

        def rows(t, h, ro, n):
            pltpu.make_async_copy(kv_h[t].at[0, h, pl.ds(mul(SK - W + ro, 16), n), :], kv_v.at[t, h, pl.ds(mul(ro, 16), n), :], s_kv.at[t, (h >> 1) & 1]).start(priority=SHORT)

        def edge_v(h, u):
            rows(1, h, (AA[1] + NA * PR + u * (PR // 8)) & (W - 1), PR // 8)

        def wait_pair(t, p):
            for u in range(2):
                @pl.when(t == u)
                def _():
                    r_ = kv_v.at[u, pl.ds(2 * p, 2), pl.ds(0, W if u == 1 and ev else NN[u] * PR + (AA[u] if ev == 2 else 0)), :]
                    pltpu.make_async_copy(r_, r_, s_kv.at[u, p & 1]).wait()

        def wo_rows(ro, n, s):
            return pltpu.make_async_copy(wo_h.at[pl.ds(ro, n), :], w_v.at[pl.ds(ro, n), :], s)

        def wo_row(n):
            return (n & 7) * BR + WO0 + (n >> 3) * WR

        def wo_copy(n):
            return wo_rows(mul(wo_row(n), 16), WR, s_wo.at[n])

        def wo_half(u):
            n = u - jnp.where(u >= N0, N0, 0)
            wo_rows(mul(wo_row(n) + jnp.where(u >= N0, WR // 2, 0), 16), WR // 2, s_wo.at[n]).start(priority=SHORT)

        def column(h, o):
            o = jnp.concatenate([o.astype(BF16).astype(F32)] * (DH // 8), axis=0)
            dg = jnp.where(jax.lax.broadcasted_iota(jnp.int32, (DH, DH), 0) == jax.lax.broadcasted_iota(jnp.int32, (DH, DH), 1), o, 0.0)
            c_v[pl.ds(mul(h * DH, DH), DH), :] = jnp.broadcast_to(jnp.sum(dg, axis=-1, keepdims=True), (DH, DH))

        def wq_piece(n):
            g = (n >> 3) + (n & 7) * 8
            for r_, c0, c1 in ((g, Q0, NH * DH), ((g + 1) & 63, 0, Q0)):
                if c1 > c0:
                    ro = mul(r_ * 8, 8)
                    pltpu.make_async_copy(wq_h.at[pl.ds(ro, 8), pl.ds(c0, c1 - c0)], wq_v.at[pl.ds(ro, 8), pl.ds(c0, c1 - c0)], s_wq).start(priority=SHORT)

        copy_x = pltpu.make_async_copy(x_h, x_v, s_x.at[0])
        copy_wr = pltpu.make_async_copy(wr_h, wr_v, s_x.at[1])
        long_e = [[pltpu.make_async_copy(kv_h[t].at[0, pl.ds(a, b - a), pl.ds(SK - W + ro, n), :], kv_v.at[t, pl.ds(a, b - a), pl.ds(ro, n), :], s_e.at[g])
                   for t in range(2) for ro, n in ([(AA[t] + j * PR, min(PR, W - AA[t] - j * PR)) for j in range(NN[t], W // PR)] if es else [(AA[t] + NN[t] * PR, W - AA[t] - NN[t] * PR)]) + [(0, AA[t])] if n and not (t == 1 and ev) and not (ev == 2 and ro == 0)] for g, (a, b) in enumerate(zip(EG, EG[1:]))]
        GO, UO, DO = NH * DH, NH * DH + F, NH * DH + 2 * F
        long_f = [[pltpu.make_async_copy(a.at[pl.ds(ro, n), :], w_v.at[pl.ds(b + ro, n), :], s_f.at[u]) for a, b in ((wg_h, GO), (wu_h, UO), (wd_h, DO))]
                  for u, (ro, n) in enumerate((a * FC, min(b * FC, F) - a * FC) for a, b in zip(FS, FS[1:] + (NF,)))]
        long_wo = [wo_copy(56 + b) for b in range(NB - 1)] + [wo_rows(a, n, s_wo.at[63]) for a, n in ((wo_row(63), WR - WO0), (0, WO0)) if n]

        jk = [pltpu.make_async_copy(k_h.at[0, pl.ds(0, 4), pl.ds(0, W), :], kv_v.at[0, pl.ds(0, 4)], s_x.at[0])] if junk else []
        longs = sum(long_e[:3], [])
        longs[0].start(priority=LONG)
        pl.delay(1)
        wq_piece(0)
        copy_x.start(priority=SHORT)
        copy_wr.start(priority=SHORT)
        pl.delay(T0 or TP - 40)
        n0 = 6
        per = -(-(len(longs) - 1) // (n0 - 1))
        for n in range(1, n0):
            wq_piece(n)
            for c in longs[1 + (n - 1) * per:1 + n * per]:
                pl.delay(1)
                c.start(priority=LONG)
            pl.delay(TP - 3 * per)
        wq_piece(n0)
        copy_x.wait()
        copy_wr.wait()
        x = x_v[0].astype(F32)
        mean = jnp.mean(x, axis=-1, keepdims=True)
        xc = x - mean
        pl.delay(TN[0])
        wq_piece(n0 + 1)
        var = jnp.mean(jnp.square(xc), axis=-1, keepdims=True)
        xn_b = (xc / jnp.sqrt(var + 1e-5)).astype(BF16)
        xn = xn_b.astype(F32)
        xn8 = jnp.broadcast_to(xn_b, (8, D))
        pl.delay(TN[1])
        wq_piece(n0 + 2)
        r = jnp.sum(xn * wr_v[...].reshape(1, D).astype(F32), axis=-1, keepdims=True)
        p_v[...] = jnp.zeros(p_v.shape, F32)
        l_v[...] = jnp.ones(l_v.shape, F32)
        pl.delay(TN[2])

        def pro1(n, c):
            wq_piece(n)
            pl.delay(TP)
            return c

        def pro2(c, carry):
            for t, b in ((0, 0), (0, 1), (1, 0)):
                piece(t, b, c, TI)
            return carry
        jax.lax.fori_loop(n0 + 3, 64, pro1, 0)
        with sc('pro2'):
            rows(0, 0, 0, AA[0])
            rows(0, 1, 0, AA[0])
            pl.delay(TP)
            rows(1, 0, AA[1] + NA * PR, PR - AA[1])
            rows(1, 0, 0, AA[1])
            pl.delay(TP)
            for c in range(DK):
                piece(1, 0, c, TI)
            jax.lax.fori_loop(DK, NA, pro2, 0)
        pltpu.make_async_copy(wq_v, wq_v, s_wq).wait()

        scale = DH ** -0.5

        def pv_slice(t, h, c, o, n):
            p = jnp.concatenate([p_v[c + u] for u in range(n)], axis=1).astype(BF16)
            return o + jnp.dot(p, load(kv_v, (t, h), c * (KS // 2), n * KS // 2), preferred_element_type=F32)

        def head(i, carry):
            def first(c):
                @pl.when(jnp.logical_and(i < NH - 2, c >= DK))
                def _():
                    piece(0, i + 2, c, TI)

            def second(c, n, e=None):
                @pl.when(i < NH - 1)
                def _():
                    piece(1, i + 1, c)
                    if e is not None:
                        edge_v(i + 1, e)

                @pl.when(i == NH - 1)
                def _():
                    wo_copy(n).start(priority=SHORT)

            def idle(c, carry):
                first(c)
                piece(1, i + 1, c, TI)
                return carry
            def third(c, n):
                @pl.when(i < NH - 2)
                def _():
                    piece(0, i + 2, c)

                @pl.when(i >= NH - 2)
                def _():
                    wo_copy(n).start(priority=SHORT)
            c0 = NA - QS * (1 + IL) - 3
            jax.lax.fori_loop(0, jnp.where(i < NH - 1, c0, 0), idle, 0)
            for g, a in enumerate(EG[:-1]):
                @pl.when(i == a)
                def _():
                    for c in long_e[g]:
                        c.wait()
                    if True:
                        for c in {1: sum(long_e[3:], []), 3: sum(long_f, []) + long_wo + jk}.get(g, []):
                            c.start(priority=LONG)
                            pl.delay(1)
            wait_pair(i & 1, i >> 1)
            hp = jnp.maximum(i - 1, 0)
            tp = jnp.minimum(i, 1)
            nf = lambda u: jnp.where(i == NH - 2, u, 6 + 2 * u)

            third(c0, nf(0))
            pl.delay(TQP if on('p') else T)
            o = jnp.zeros((8, DH), F32)
            if on('p'):
                l_v[...] = jnp.broadcast_to(jnp.sum(l_v[...], axis=-1, keepdims=True), (8, DH))
                q_v[...] = jnp.dot(xn8, load(wq_v, (), 0, D, pl.ds(pl.multiple_of(i * DH, DH), DH)), preferred_element_type=F32)
                o = pv_slice(tp, hp, 4, o, 2)
            second(c0, 7)
            pl.delay(1 if on('p') else T)

            def att(c, carry):
                o = carry
                third(c0 + 1 + c, nf(1 + c))

                @pl.when(i < NH - 1)
                def _():
                    edge_v(i + 1, 2 * c)
                pl.delay(TA[0] if on('a') else T)
                if on('a'):
                    s = jax.lax.dot_general(q_v[...].astype(BF16), load(kv_v, (0, i), c * KS, KS), _NT, preferred_element_type=F32)
                    o = pv_slice(tp, hp, c, o, 1)
                second(c0 + 1 + c, 9 + 2 * c, 2 * c + 1)
                if on('a'):
                    s_v[c] = s
                pl.delay(TA[1] if on('a') else T)
                if IL:
                    @pl.when(i < NH - 1)
                    def _():
                        idle(c0 + 1 + QS + c, 0)
                return o
            o = jax.lax.fori_loop(0, QS, att, o)

            third(NA - 2, nf(5))
            if KE < AA[0]:
                @pl.when(i < NH - 2)
                def _():
                    rows(0, i + 2, KE, AA[0] - KE)
            mx = None
            for c in range(QS):
                s = s_v[c] * scale
                for u in range(KS // DH):
                    mx = s[:, u * DH:(u + 1) * DH] if mx is None else jnp.maximum(mx, s[:, u * DH:(u + 1) * DH])
            pl.delay(TM if on('m') else T)
            if on('m'):
                q_v[...] = jnp.broadcast_to(jnp.max(mx, axis=-1, keepdims=True), (8, DH))
                o = pv_slice(tp, hp, 6, o, 2)
            second(NA - 2, 17)
            pl.delay(1 if on('m') else T)

            @pl.when(i < NH - 2)
            def _():
                piece(0, i + 2, NA - 1)
                rows(0, i + 2, 0, KE)
            if on('c'):
                column(hp, o / l_v[...])
            pl.delay(TC if on('c') else T)

            @pl.when(i < NH - 1)
            def _():
                piece(1, i + 1, NA - 1)
                pl.delay(TE if on('e') else T)
            if on('e'):
                tot = jnp.zeros((8, DH), F32)
                m = jnp.concatenate([q_v[...]] * (KS // DH), axis=1)
                for c in range(QS):
                    p = jnp.exp(s_v[c] * scale - m)
                    p_v[2 * c] = p[:, :KS // 2]
                    p_v[2 * c + 1] = p[:, KS // 2:]
                    for u in range(KS // DH):
                        tot = tot + p[:, u * DH:(u + 1) * DH]
                l_v[...] = tot
            return carry
        with sc('loop'):
            jax.lax.fori_loop(0, NH, head, 0)

        with sc('fwait'):
            for c in long_f[0]:
                c.wait()

        def proj(ro, n, part):
            prod = load(w_v, (), ro, n).astype(F32) * jnp.concatenate([c_v[pl.ds(mul(ro, 8), n), :]] * (D // DH), axis=1)
            return part + prod.reshape(n // 8, 8, D).sum(axis=0)

        def one(n, part):
            wo_copy(n).wait()
            return proj(wo_row(n), WR, part)

        def ffn(j, carry):
            hid, y, o, part = carry
            f0 = jnp.minimum(j * FC, F - FC)
            fp = jnp.maximum((j - 1) * FC, 0)
            wo_copy(N0 + 2 * j).start(priority=SHORT)

            for u in range(1, len(FS)):
                @pl.when(j == FS[u])
                def _():
                    for c in long_f[u]:
                        c.wait()
            for u in range(FP):
                wo_copy(FP * j + u).wait()
            pl.delay(TF[0])
            gt = jax.lax.dot_general(xn8, load(w_v, (), GO + f0, FC), _NT, preferred_element_type=F32)
            up = jax.lax.dot_general(xn8, load(w_v, (), UO + f0, FC), _NT, preferred_element_type=F32)
            o = jnp.where(j < 2 * QS, pv_slice(1, NH - 1, jnp.minimum(j, 2 * QS - 1), o, 1), o)
            t = jnp.dot(hid.astype(BF16), load(w_v, (), DO + fp, FC), preferred_element_type=F32)
            wo_copy(N0 + 1 + 2 * j).start(priority=SHORT)
            for u in range(FP):
                part = proj(wo_row(FP * j + u), WR, part)
            col = f0 + jax.lax.broadcasted_iota(jnp.int32, (8, FC), 1)
            hid = jnp.where(col >= j * FC, jax.nn.silu(gt) * up, 0.0)
            y = jnp.where(j > 0, y + t, y)
            pl.delay(TF[1])
            return hid, y, o, part
        zd = jnp.zeros((8, D), F32)
        with sc('ffn'):
            hid, y, o, part = jax.lax.fori_loop(0, NF, ffn, (jnp.zeros((8, FC), F32), zd, jnp.zeros((8, DH), F32), zd))
        n1 = N0 + 2 * NF
        wo_copy(n1).start(priority=SHORT)
        q_v[...] = o / jnp.sum(l_v[...], axis=-1, keepdims=True)
        y = y + jnp.dot(hid.astype(BF16), load(w_v, (), DO + F - FC, FC), preferred_element_type=F32)
        pl.delay(TG[0])
        wo_copy(n1 + 1).start(priority=SHORT)
        column(NH - 1, q_v[...])
        gate = jax.nn.silu(xn + (xn * 0.0 + y * jax.nn.sigmoid(r)))
        pl.delay(TG[1])

        ns = 55 - n1 - 2

        def slot(c, part):
            wo_copy(n1 + 2 + c).start(priority=SHORT)
            part = one(FP * NF + 2 * c + 1, one(FP * NF + 2 * c, part))
            part = jax.lax.fori_loop(0, (c >= ns - WP).astype(jnp.int32), lambda u, t: one(56 + c - ns + WP, t), part)
            pl.delay(TW)
            return part
        with sc('proj'):
            part = jax.lax.fori_loop(0, ns, slot, part)
        a_ = wo_row(55)
        tail = [(a_, WR - last), (a_ + WR - last, last)] if last else [(a_, WR)]
        tc = [wo_rows(a, n, s_wo.at[(55, 64)[c]]) for c, (a, n) in enumerate(tail)]
        for c in tc:
            c.start(priority=SHORT)
            pl.delay(1)
        n2 = FP * NF + 2 * ns
        part = jax.lax.fori_loop(n2, WL + NB - 1 - WP, lambda n, t: one(jnp.where(n < WL, n, n - WL + 56 + WP), t), part)
        with sc('wwait'):
            for c in long_wo[NB - 1:]:
                c.wait()
        part = proj(NH * DH - WR + WO0, WR - WO0, proj(0, WO0, part) if WO0 else part)
        with sc('one'):
            part = jax.lax.fori_loop(WL, 55, one, part)
        for c, (a, n) in enumerate(tail):
            with sc(f't{c}'):
                tc[c].wait()
            part = proj(a, n, part)
        for c in jk:
            c.wait()
        s_out = jnp.sum(part, axis=0, keepdims=True)
        res = jnp.broadcast_to(x, (8, D)) + jnp.broadcast_to(s_out, (8, D)) * gate
        out_ref[0] = res.astype(out_ref.dtype)[0:1]

    def fn(A_x, A_k_cache, A_v_cache, A_wq, A_wo, B_x, B_w_r, B_w_gate, B_w_up, B_w_down):
        hbm = pl.BlockSpec(memory_space=pltpu.HBM)
        dma = pltpu.SemaphoreType.DMA
        V = pltpu.VMEM
        return pl.pallas_call(
            kernel, name=name, out_shape=jax.ShapeDtypeStruct((1, 1, D), BF16), in_specs=[hbm] * 9,
            out_specs=pl.BlockSpec(memory_space=pltpu.VMEM),
            scratch_shapes=[V((1, 1, D), BF16), V((D,), BF16), V((D, NH * DH), BF16), V((2, NH, W, DH), BF16), V((NH * DH + 3 * F, D), BF16),
                            V((8, DH), F32), V((QS, 8, KS), F32), V((2 * QS, 8, KS // 2), F32), V((8, DH), F32), V((NH * DH, DH), F32),
                            dma((2,)), dma, dma((len(FS),)), dma((2, 2)), dma((len(EG) - 1,)), dma((65,))],
            compiler_params=pltpu.CompilerParams(vmem_limit_bytes=100 * 1024 * 1024, disable_semaphore_checks=True, disable_bounds_checks=nbc),
        )(A_x, A_k_cache, A_v_cache, A_wq, A_wo, B_w_r, B_w_gate.T, B_w_up.T, B_w_down)
    return fn


pallas_recurrent_scan__sliding_block_cached__moe_arch_mod__decode_kernel = jax.jit(build(TP=89,WP=4))
```

```python
import jax
import jax.numpy as jnp
import jax.experimental.pallas as pl
import jax.experimental.pallas.tpu as pltpu

D = 512
NH = 32
DH = 128
SK = 32768
W = min(4096, max(256, SK // 4))
F = 1376

KV0 = (128, 64)
WQ0 = 2048
WO0 = 32

PR = 256
NA = W // PR - 1
ER = PR // 8
NP = (11, NA)
K_GROUPS = (0, 2, 4, 8, 13, 19, 25, 32)
WR = 64
QS = 4
KS = W // QS
VS = KS // 2
FC = 128
NF = -(-F // FC)
F_GROUPS = (0, 7, 10, NF)
N_FILL = 20
N_PACED = 56
N_SPLIT = 8
LAST = 16
GO, UO, DO = NH * DH, NH * DH + F, NH * DH + 2 * F

T_KV, T_WQ, T_FIRST, T_NORM = 94, 92, 100, (80, 40, 60)
T_Q, T_ATT, T_MAX, T_COL, T_EXP, T_WO, T_SPLIT = 14, 4, 30, 8, 56, 50, 18

BF16 = jnp.bfloat16
F32 = jnp.float32
_NT = (((1,), (1,)), ((), ()))
LONG, SHORT = 1, 0


def _mul(a, m):
    return a if isinstance(a, int) else pl.multiple_of(a, m)


def _kernel(x_h, k_h, v_h, wq_h, wo_h, wr_h, wg_h, wu_h, wd_h, out_ref,
            x_v, wr_v, wq_v, kv_v, w_v, q_v, s_v, p_v, l_v, c_v, s_x, s_wq, s_f, s_kv, s_k, s_wo):
    kv_h = (k_h, v_h)

    def start_rows(t, h, ro, n):
        pltpu.make_async_copy(kv_h[t].at[0, h, pl.ds(_mul(SK - W + ro, 16), n), :],
                              kv_v.at[t, h, pl.ds(_mul(ro, 16), n), :],
                              s_kv.at[t, (h >> 1) & 1]).start(priority=SHORT)

    def start_piece(t, u, c):
        n = (u & 1) * NP[t] + c - (NA - NP[t])
        j = n >> 1
        start_rows(t, (u & ~1) + (n & 1), KV0[t] + ((j >> 1) + (j & 1) * ((NP[t] + 1) // 2)) * PR, PR)

    def start_edge(t, h, e, n):
        start_rows(t, h, (KV0[t] + NA * PR + e * ER) & (W - 1), n * ER)

    def wait_pair(t, p):
        k0, k1 = KV0[t] + NP[t] * PR, KV0[t] + NA * PR
        for a, b in ((0, k0), (k1, W)) if k1 > k0 else ((0, W),):
            rows = kv_v.at[t, pl.ds(2 * p, 2), pl.ds(a, b - a), :]
            pltpu.make_async_copy(rows, rows, s_kv.at[t, p & 1]).wait()

    def wo_rows(ro, n, s):
        return pltpu.make_async_copy(wo_h.at[pl.ds(_mul(ro, 16), n), :], w_v.at[pl.ds(_mul(ro, 16), n), :],
                                     s_wo.at[s])

    def wo_row(n):
        return (n & 7) * 8 * WR + WO0 + (n >> 3) * WR

    def wo_piece(n):
        return wo_rows(wo_row(n), WR, n)

    def start_wq(n):
        g = (n >> 3) + (n & 7) * 8
        for r, c0, c1 in ((g, WQ0, NH * DH), ((g + 1) & 63, 0, WQ0)):
            if c1 > c0:
                idx = (pl.ds(_mul(r * 8, 8), 8), pl.ds(c0, c1 - c0))
                pltpu.make_async_copy(wq_h.at[idx], wq_v.at[idx], s_wq).start(priority=SHORT)

    def start_long(copies):
        for c in copies:
            c.start(priority=LONG)
            pl.delay(1)

    copy_x = pltpu.make_async_copy(x_h, x_v, s_x.at[0])
    copy_wr = pltpu.make_async_copy(wr_h, wr_v, s_x.at[1])
    k0, kn = KV0[0] + NP[0] * PR, (NA - NP[0]) * PR
    long_k = [pltpu.make_async_copy(k_h.at[0, pl.ds(a, b - a), pl.ds(SK - W + k0, kn), :],
                                    kv_v.at[0, pl.ds(a, b - a), pl.ds(k0, kn), :], s_k.at[g])
              for g, (a, b) in enumerate(zip(K_GROUPS, K_GROUPS[1:]))]
    long_f = [[pltpu.make_async_copy(src.at[pl.ds(a * FC, min(b * FC, F) - a * FC), :],
                                     w_v.at[pl.ds(o + a * FC, min(b * FC, F) - a * FC), :], s_f.at[g])
               for src, o in ((wg_h, GO), (wu_h, UO), (wd_h, DO))]
              for g, (a, b) in enumerate(zip(F_GROUPS, F_GROUPS[1:]))]
    wrap = [(a, n) for a, n in ((wo_row(63), WR - WO0), (0, WO0)) if n]

    def wq_slot(n, carry):
        start_wq(n)
        pl.delay(T_WQ)
        return carry

    start_long(long_k[:1])
    start_wq(0)
    copy_x.start(priority=SHORT)
    copy_wr.start(priority=SHORT)
    pl.delay(T_FIRST)
    jax.lax.fori_loop(1, 6, wq_slot, 0)

    start_wq(6)
    copy_x.wait()
    copy_wr.wait()
    x = x_v[0].astype(F32)
    xc = x - jnp.mean(x, axis=-1, keepdims=True)
    pl.delay(T_NORM[0])
    start_wq(7)
    var = jnp.mean(jnp.square(xc), axis=-1, keepdims=True)
    xn_b = (xc / jnp.sqrt(var + 1e-5)).astype(BF16)
    xn = xn_b.astype(F32)
    xn8 = jnp.broadcast_to(xn_b, (8, D))
    pl.delay(T_NORM[1])
    start_wq(8)
    r = jnp.sum(xn * wr_v[...].reshape(1, D).astype(F32), axis=-1, keepdims=True)
    p_v[...] = jnp.zeros(p_v.shape, F32)
    l_v[...] = jnp.ones(l_v.shape, F32)
    pl.delay(T_NORM[2])

    start_long(long_k[1:])
    jax.lax.fori_loop(9, 64 - 3 * NP[0], wq_slot, 0)
    ahead = ((0, 0), (0, 1), (1, 0))
    for t, h in ahead:
        for e in range(0, 8, 2):
            start_edge(t, h, e, 2)
        pl.delay(T_WQ)
    for c in range(NA - NP[0]):
        start_piece(1, 0, c)
        pl.delay(T_KV)

    def lead(c, carry):
        for u, (t, b) in enumerate(ahead):
            wq_slot(64 - 3 * (NA - c) + u, 0)
            start_piece(t, b, c)
            pl.delay(T_KV)
        return carry

    jax.lax.fori_loop(NA - NP[0], NA, lead, 0)

    scale = DH ** -0.5

    def pv(t, h, c, n, o):
        p = jnp.concatenate([p_v[c + u] for u in range(n)], axis=1).astype(BF16)
        return o + jnp.dot(p, kv_v[t, h, pl.ds(_mul(c * VS, VS), n * VS), :], preferred_element_type=F32)

    def column(h, o):
        o = jnp.concatenate([o.astype(BF16).astype(F32)] * (DH // 8), axis=0)
        eye = (jax.lax.broadcasted_iota(jnp.int32, (DH, DH), 0)
               == jax.lax.broadcasted_iota(jnp.int32, (DH, DH), 1))
        col = jnp.sum(jnp.where(eye, o, 0.0), axis=-1, keepdims=True)
        c_v[pl.ds(_mul(h * DH, DH), DH), :] = jnp.broadcast_to(col, (DH, DH))

    def head(i, carry):
        def issue(t, c, n, edge=None):
            @pl.when(i + 2 - t < NH)
            def _():
                start_piece(t, i + 2 - t, c)
                if edge is not None:
                    start_edge(t, i + 2 - t, *edge)

            @pl.when(i + 2 - t >= NH)
            def _():
                wo_piece(n).start(priority=SHORT)

        def fill(u):
            return jnp.where(i == NH - 2, u, 7 + 2 * u)

        def idle(c, carry):
            @pl.when(jnp.logical_and(i + 2 < NH, c >= NA - NP[0]))
            def _():
                start_piece(0, i + 2, c)
                pl.delay(T_KV)
            start_piece(1, i + 1, c)
            pl.delay(T_KV)
            return carry

        c0 = NA - QS - 3
        jax.lax.fori_loop(0, jnp.where(i + 1 < NH, c0, 0), idle, 0)
        for g, a in enumerate(K_GROUPS[:-1]):
            @pl.when(i == a)
            def _():
                long_k[g].wait()
                if g == 0:
                    pltpu.make_async_copy(wq_v, wq_v, s_wq).wait()
                if g == 4:
                    start_long(sum(long_f, []) + [wo_piece(n) for n in range(N_PACED, 63)]
                               + [wo_rows(a_, n, 63) for a_, n in wrap])
        for t in range(2):
            @pl.when((i & 1) == t)
            def _():
                wait_pair(t, i >> 1)
        hp = jnp.maximum(i - 1, 0)
        tp = jnp.minimum(i, 1)

        issue(0, c0, fill(0))
        pl.delay(T_Q)
        l_v[...] = jnp.broadcast_to(jnp.sum(l_v[...], axis=-1, keepdims=True), (8, DH))
        q_v[...] = jnp.dot(xn8, wq_v[:, pl.ds(pl.multiple_of(i * DH, DH), DH)], preferred_element_type=F32)
        o = pv(tp, hp, 4, 2, jnp.zeros((8, DH), F32))
        issue(1, c0, 8)
        pl.delay(1)

        def att(c, o):
            issue(0, c0 + 1 + c, fill(1 + c), (c, 1))
            pl.delay(T_ATT)
            s = jax.lax.dot_general(q_v[...].astype(BF16), kv_v[0, i, pl.ds(pl.multiple_of(c * KS, KS), KS), :],
                                    _NT, preferred_element_type=F32)
            o = pv(tp, hp, c, 1, o)
            issue(1, c0 + 1 + c, 10 + 2 * c, (c, 1))
            s_v[c] = s
            pl.delay(1)
            return o

        o = jax.lax.fori_loop(0, QS, att, o)

        issue(0, NA - 2, fill(5), (4, 2))
        mx = None
        for c in range(QS):
            s = s_v[c] * scale
            for u in range(0, KS, DH):
                mx = s[:, u:u + DH] if mx is None else jnp.maximum(mx, s[:, u:u + DH])
        pl.delay(T_MAX)
        q_v[...] = jnp.broadcast_to(jnp.max(mx, axis=-1, keepdims=True), (8, DH))
        o = pv(tp, hp, 6, 2, o)
        issue(1, NA - 2, 18, (4, 2))
        pl.delay(1)

        issue(0, NA - 1, fill(6), (6, 2))
        column(hp, o / l_v[...])
        pl.delay(T_COL)

        @pl.when(i + 1 < NH)
        def _():
            start_piece(1, i + 1, NA - 1)
            start_edge(1, i + 1, 6, 2)
            pl.delay(T_EXP)
        tot = jnp.zeros((8, DH), F32)
        m = jnp.concatenate([q_v[...]] * (KS // DH), axis=1)
        for c in range(QS):
            p = jnp.exp(s_v[c] * scale - m)
            p_v[2 * c] = p[:, :VS]
            p_v[2 * c + 1] = p[:, VS:]
            for u in range(0, KS, DH):
                tot = tot + p[:, u:u + DH]
        l_v[...] = tot
        return carry

    jax.lax.fori_loop(0, NH, head, 0)

    def proj(ro, n, part):
        coef = jnp.concatenate([c_v[pl.ds(_mul(ro, 16), n), :]] * (D // DH), axis=1)
        prod = w_v[pl.ds(_mul(ro, 16), n), :].astype(F32) * coef
        return part + prod.reshape(n // 8, 8, D).sum(axis=0)

    def proj_piece(n, part):
        wo_piece(n).wait()
        return proj(wo_row(n), WR, part)

    def w_rows(ro):
        return w_v[pl.ds(_mul(ro, 16), FC), :]

    def ffn(j, carry):
        hid, y, o, part = carry
        f0 = jnp.minimum(j * FC, F - FC)
        wo_piece(N_FILL + 2 * j).start(priority=SHORT)
        for g, a in enumerate(F_GROUPS[:-1]):
            @pl.when(j == a)
            def _():
                for c in long_f[g]:
                    c.wait()
        for u in range(2):
            wo_piece(2 * j + u).wait()
        pl.delay(1)
        gt = jax.lax.dot_general(xn8, w_rows(GO + f0), _NT, preferred_element_type=F32)
        up = jax.lax.dot_general(xn8, w_rows(UO + f0), _NT, preferred_element_type=F32)
        o = jnp.where(j < 2 * QS, pv(1, NH - 1, jnp.minimum(j, 2 * QS - 1), 1, o), o)
        t = jnp.dot(hid.astype(BF16), w_rows(DO + jnp.maximum(j - 1, 0) * FC), preferred_element_type=F32)
        wo_piece(N_FILL + 2 * j + 1).start(priority=SHORT)
        for u in range(2):
            part = proj(wo_row(2 * j + u), WR, part)
        col = f0 + jax.lax.broadcasted_iota(jnp.int32, (8, FC), 1)
        hid = jnp.where(col >= j * FC, jax.nn.silu(gt) * up, 0.0)
        y = jnp.where(j > 0, y + t, y)
        pl.delay(1)
        return hid, y, o, part

    zero = jnp.zeros((8, D), F32)
    hid, y, o, part = jax.lax.fori_loop(
        0, NF, ffn, (jnp.zeros((8, FC), F32), zero, jnp.zeros((8, DH), F32), zero))
    n1 = N_FILL + 2 * NF
    wo_piece(n1).start(priority=SHORT)
    q_v[...] = o / jnp.sum(l_v[...], axis=-1, keepdims=True)
    y = y + jnp.dot(hid.astype(BF16), w_rows(DO + F - FC), preferred_element_type=F32)
    pl.delay(1)
    wo_piece(n1 + 1).start(priority=SHORT)
    column(NH - 1, q_v[...])
    gate = jax.nn.silu(xn + (xn * 0.0 + y * jax.nn.sigmoid(r)))
    pl.delay(1)

    lag = 2 * (n1 + 2) - 2 * NF

    def slot(n, part):
        wo_piece(n).start(priority=SHORT)
        part = proj_piece(2 * n - lag + 1, proj_piece(2 * n - lag, part))
        pl.delay(T_WO)
        return part

    def split_slot(n, part):
        for e, prio in enumerate((SHORT, LONG)):
            wo_rows(wo_row(n) + e * (WR // 2), WR // 2, n).start(priority=prio)
            part = proj_piece(2 * n - lag + e, part)
            pl.delay(T_SPLIT)
        return part

    n2, n3 = N_PACED - N_SPLIT, N_PACED - 1
    part = jax.lax.fori_loop(n1 + 2, n2, slot, part)
    part = jax.lax.fori_loop(n2, n3, split_slot, part)
    tail = ((wo_row(n3), WR - LAST, n3), (wo_row(n3) + WR - LAST, LAST, 64))
    for rows, prio in zip(tail, (SHORT, LONG)):
        wo_rows(*rows).start(priority=prio)
        pl.delay(1)
    for n in list(range(2 * n3 - lag, n2)) + list(range(N_PACED, 63)):
        part = proj_piece(n, part)
    for a, n in wrap:
        wo_rows(a, n, 63).wait()
    for a, n in wrap:
        part = proj(a, n, part)
    for n in range(n2, n3):
        part = proj_piece(n, part)
    for a, n, s in tail:
        wo_rows(a, n, s).wait()
        part = proj(a, n, part)
    s_out = jnp.sum(part, axis=0, keepdims=True)

    res = jnp.broadcast_to(x, (8, D)) + jnp.broadcast_to(s_out, (8, D)) * gate
    out_ref[0] = res.astype(out_ref.dtype)[0:1]


@jax.jit
def pallas_recurrent_scan__sliding_block_cached__moe_arch_mod__decode_kernel(
    A_x: jax.Array,
    A_k_cache: jax.Array,
    A_v_cache: jax.Array,
    A_wq: jax.Array,
    A_wo: jax.Array,
    B_x: jax.Array,
    B_w_r: jax.Array,
    B_w_gate: jax.Array,
    B_w_up: jax.Array,
    B_w_down: jax.Array,
):
    del B_x
    hbm = pl.BlockSpec(memory_space=pltpu.HBM)
    dma = pltpu.SemaphoreType.DMA
    return pl.pallas_call(
        _kernel,
        out_shape=jax.ShapeDtypeStruct((1, 1, D), BF16),
        in_specs=[hbm] * 9,
        out_specs=pl.BlockSpec(memory_space=pltpu.VMEM),
        scratch_shapes=[
            pltpu.VMEM((1, 1, D), BF16),
            pltpu.VMEM((D,), BF16),
            pltpu.VMEM((D, NH * DH), BF16),
            pltpu.VMEM((2, NH, W, DH), BF16),
            pltpu.VMEM((NH * DH + 3 * F, D), BF16),
            pltpu.VMEM((8, DH), F32),
            pltpu.VMEM((QS, 8, KS), F32),
            pltpu.VMEM((2 * QS, 8, VS), F32),
            pltpu.VMEM((8, DH), F32),
            pltpu.VMEM((NH * DH, DH), F32),
            dma((2,)), dma, dma((len(F_GROUPS) - 1,)), dma((2, 2)), dma((len(K_GROUPS) - 1,)), dma((65,)),
        ],
        compiler_params=pltpu.CompilerParams(
            vmem_limit_bytes=100 * 1024 * 1024,
            disable_semaphore_checks=True,
            disable_bounds_checks=True,
        ),
    )(A_x, A_k_cache, A_v_cache, A_wq, A_wo, B_w_r, B_w_gate.T, B_w_up.T, B_w_down)
```

```python
import jax
import jax.numpy as jnp
import jax.experimental.pallas as pl
import jax.experimental.pallas.tpu as pltpu

D = 512
NH = 32
DH = 128
SK = 32768
W = min(4096, max(256, SK // 4))
F = 1376

KV0 = (128, 64)
WQ0 = 2048
WO0 = 32

PR = 256
NA = W // PR - 1
ER = PR // 8
NP = (12, NA)
K_GROUPS = (0, 2, 6, 12, 18, 25, 32)
WQ_LONG = 3
WR = 64
QS = 4
KS = W // QS
VS = KS // 2
FC = 128
NF = -(-F // FC)
F_GROUPS = (0, 7, 10, NF)
N_FILL = 20
N_PACED = 56
N_SPLIT = 4
LAST = 16
FP = 3
GO, UO, DO = NH * DH, NH * DH + F, NH * DH + 2 * F

T_KV, T_WQ, T_EDGE, T_FIRST, T_NORM = (44, 45), 45, 22, 100, (35, 1, 15)
T_Q, T_ATT, T_MAX, T_EXP, T_WO, T_SPLIT = 10, 5, 16, 46, 24, 14

BF16 = jnp.bfloat16
F32 = jnp.float32
_NT = (((1,), (1,)), ((), ()))
LONG, SHORT = 1, 0


def _mul(a, m):
    return a if isinstance(a, int) else pl.multiple_of(a, m)


def _kernel(x_h, k_h, v_h, wq_h, wo_h, wr_h, wg_h, wu_h, wd_h, out_ref,
            x_v, wr_v, wq_v, kv_v, w_v, q_v, s_v, p_v, l_v, c_v, s_x, s_wq, s_f, s_kv, s_k, s_wo):
    kv_h = (k_h, v_h)

    def start_rows(t, h, ro, n):
        pltpu.make_async_copy(kv_h[t].at[0, h, pl.ds(_mul(SK - W + ro, 16), n), :],
                              kv_v.at[t, h, pl.ds(_mul(ro, 16), n), :],
                              s_kv.at[t, (h >> 1) & 1]).start(priority=SHORT)

    def start_piece(t, u, c, idle=False):
        n = (u & 1) * NP[t] + c - (NA - NP[t])
        j = n >> 1
        h, ro = (u & ~1) + (n & 1), KV0[t] + ((j >> 1) + (j & 1) * ((NP[t] + 1) // 2)) * PR
        if idle:
            for e in range(2):
                start_rows(t, h, ro + e * PR // 2, PR // 2)
                pl.delay(T_KV[e])
        else:
            start_rows(t, h, ro, PR)

    def start_edge(t, h, e, n):
        start_rows(t, h, (KV0[t] + NA * PR + e * ER) & (W - 1), n * ER)

    def wait_pair(t, p):
        k0, k1 = KV0[t] + NP[t] * PR, KV0[t] + NA * PR
        for a, b in ((0, k0), (k1, W)) if k1 > k0 else ((0, W),):
            rows = kv_v.at[t, pl.ds(2 * p, 2), pl.ds(a, b - a), :]
            pltpu.make_async_copy(rows, rows, s_kv.at[t, p & 1]).wait()

    def wo_rows(ro, n, s):
        return pltpu.make_async_copy(wo_h.at[pl.ds(_mul(ro, 16), n), :], w_v.at[pl.ds(_mul(ro, 16), n), :],
                                     s_wo.at[s])

    def wo_row(n):
        return (n & 7) * 8 * WR + WO0 + (n >> 3) * WR

    def wo_piece(n):
        return wo_rows(wo_row(n), WR, n)

    def start_wq(n, pause=0, prio=SHORT):
        g = (n >> 3) + (n & 7) * 8
        for r, c0, c1 in ((g, WQ0, NH * DH), ((g + 1) & 63, 0, WQ0)):
            if c1 > c0:
                idx = (pl.ds(_mul(r * 8, 8), 8), pl.ds(c0, c1 - c0))
                pltpu.make_async_copy(wq_h.at[idx], wq_v.at[idx], s_wq).start(priority=prio)
            if pause and c1 == NH * DH:
                pl.delay(pause)

    def start_long(copies):
        for c in copies:
            c.start(priority=LONG)
            pl.delay(1)

    copy_x = pltpu.make_async_copy(x_h, x_v, s_x.at[0])
    copy_wr = pltpu.make_async_copy(wr_h, wr_v, s_x.at[1])
    long_k = [[pltpu.make_async_copy(k_h.at[0, pl.ds(a, b - a), pl.ds(SK - W + KV0[0] + j * PR, PR), :],
                                     kv_v.at[0, pl.ds(a, b - a), pl.ds(KV0[0] + j * PR, PR), :], s_k.at[g])
               for j in range(NP[0], NA)]
              for g, (a, b) in enumerate(zip(K_GROUPS, K_GROUPS[1:]))]
    long_f = [[pltpu.make_async_copy(src.at[pl.ds(a * FC, min(b * FC, F) - a * FC), :],
                                     w_v.at[pl.ds(o + a * FC, min(b * FC, F) - a * FC), :], s_f.at[g])
               for src, o in ((wg_h, GO), (wu_h, UO), (wd_h, DO))]
              for g, (a, b) in enumerate(zip(F_GROUPS, F_GROUPS[1:]))]
    wrap = [(a, n) for a, n in ((wo_row(63), WR - WO0), (0, WO0)) if n]

    def wq_slot(n, carry):
        start_wq(n, T_WQ)
        pl.delay(T_WQ)
        return carry

    start_long(long_k[0])
    start_wq(0)
    copy_x.start(priority=SHORT)
    copy_wr.start(priority=SHORT)
    pl.delay(T_FIRST)
    jax.lax.fori_loop(1, 6, wq_slot, 0)

    start_wq(6, T_WQ)
    copy_x.wait()
    copy_wr.wait()
    x = x_v[0].astype(F32)
    xc = x - jnp.mean(x, axis=-1, keepdims=True)
    pl.delay(T_NORM[0])
    start_wq(7, T_WQ)
    var = jnp.mean(jnp.square(xc), axis=-1, keepdims=True)
    xn_b = (xc / jnp.sqrt(var + 1e-5)).astype(BF16)
    xn = xn_b.astype(F32)
    xn8 = jnp.broadcast_to(xn_b, (8, D))
    pl.delay(T_NORM[1])
    start_wq(8, T_WQ)
    r = jnp.sum(xn * wr_v[...].reshape(1, D).astype(F32), axis=-1, keepdims=True)
    p_v[...] = jnp.zeros(p_v.shape, F32)
    l_v[...] = jnp.ones(l_v.shape, F32)
    pl.delay(T_NORM[2])

    for n in range(WQ_LONG):
        start_wq(9 + n, prio=LONG)
    pl.delay(1)
    start_long(sum(long_k[1:], []))
    jax.lax.fori_loop(9 + WQ_LONG, 64 - 3 * NP[0], wq_slot, 0)
    ahead = ((0, 0), (0, 1), (1, 0))
    for t, h in ahead:
        for e in range(0, 8, 2):
            start_edge(t, h, e, 2)
            pl.delay(T_EDGE)
    for c in range(NA - NP[0]):
        start_piece(1, 0, c, idle=True)

    def lead(c, carry):
        for u, (t, b) in enumerate(ahead):
            wq_slot(64 - 3 * (NA - c) + u, 0)
            start_piece(t, b, c, idle=True)
        return carry

    jax.lax.fori_loop(NA - NP[0], NA, lead, 0)

    scale = DH ** -0.5

    def pv(t, h, c, n, o):
        p = jnp.concatenate([p_v[c + u] for u in range(n)], axis=1).astype(BF16)
        return o + jnp.dot(p, kv_v[t, h, pl.ds(_mul(c * VS, VS), n * VS), :], preferred_element_type=F32)

    def column(h, o):
        o = jnp.concatenate([o.astype(BF16).astype(F32)] * (DH // 8), axis=0)
        eye = (jax.lax.broadcasted_iota(jnp.int32, (DH, DH), 0)
               == jax.lax.broadcasted_iota(jnp.int32, (DH, DH), 1))
        col = jnp.sum(jnp.where(eye, o, 0.0), axis=-1, keepdims=True)
        c_v[pl.ds(_mul(h * DH, DH), DH), :] = jnp.broadcast_to(col, (DH, DH))

    def head(i, carry):
        def issue(t, c, n, edge=None):
            @pl.when(i + 2 - t < NH)
            def _():
                start_piece(t, i + 2 - t, c)
                if edge is not None:
                    start_edge(t, i + 2 - t, *edge)

            @pl.when(i + 2 - t >= NH)
            def _():
                wo_piece(n).start(priority=SHORT)

        def fill(u):
            return jnp.where(i == NH - 2, u, 7 + 2 * u)

        def idle(c, carry):
            @pl.when(jnp.logical_and(i + 2 < NH, c >= NA - NP[0]))
            def _():
                start_piece(0, i + 2, c, idle=True)
            start_piece(1, i + 1, c, idle=True)
            return carry

        c0 = NA - QS - 3
        jax.lax.fori_loop(0, jnp.where(i + 1 < NH, c0, 0), idle, 0)
        for g, a in enumerate(K_GROUPS[:-1]):
            @pl.when(i == a)
            def _():
                for c in long_k[g]:
                    c.wait()
                if g == 0:
                    pltpu.make_async_copy(wq_v, wq_v, s_wq).wait()
                if g == 4:
                    start_long(sum(long_f, []) + [wo_piece(n) for n in range(N_PACED, 63)]
                               + [wo_rows(a_, n, 63) for a_, n in wrap])
        for t in range(2):
            @pl.when((i & 1) == t)
            def _():
                wait_pair(t, i >> 1)
        hp = jnp.maximum(i - 1, 0)
        tp = jnp.minimum(i, 1)

        issue(0, c0, fill(0))
        pl.delay(T_Q)
        l_v[...] = jnp.broadcast_to(jnp.sum(l_v[...], axis=-1, keepdims=True), (8, DH))
        q_v[...] = jnp.dot(xn8, wq_v[:, pl.ds(pl.multiple_of(i * DH, DH), DH)], preferred_element_type=F32)
        o = pv(tp, hp, 4, 2, jnp.zeros((8, DH), F32))
        issue(1, c0, 8)
        pl.delay(1)

        def att(c, o):
            issue(0, c0 + 1 + c, fill(1 + c), (c, 1))
            pl.delay(T_ATT)
            s = jax.lax.dot_general(q_v[...].astype(BF16), kv_v[0, i, pl.ds(pl.multiple_of(c * KS, KS), KS), :],
                                    _NT, preferred_element_type=F32)
            o = pv(tp, hp, c, 1, o)
            issue(1, c0 + 1 + c, 10 + 2 * c, (c, 1))
            s_v[c] = s
            pl.delay(1)
            return o

        o = jax.lax.fori_loop(0, QS, att, o)

        issue(0, NA - 2, fill(5))
        mx = None
        for c in range(QS):
            s = s_v[c] * scale
            for u in range(0, KS, DH):
                mx = s[:, u:u + DH] if mx is None else jnp.maximum(mx, s[:, u:u + DH])
        pl.delay(T_MAX)

        @pl.when(i + 2 < NH)
        def _():
            start_edge(0, i + 2, 4, 2)
        pl.delay(1)
        q_v[...] = jnp.broadcast_to(jnp.max(mx, axis=-1, keepdims=True), (8, DH))
        o = pv(tp, hp, 6, 2, o)
        issue(1, NA - 2, 18, (4, 2))
        pl.delay(1)

        issue(0, NA - 1, fill(6), (6, 2))
        column(hp, o / l_v[...])
        pl.delay(1)

        @pl.when(i + 1 < NH)
        def _():
            start_piece(1, i + 1, NA - 1)
            start_edge(1, i + 1, 6, 2)
            pl.delay(T_EXP)
        tot = jnp.zeros((8, DH), F32)
        m = jnp.concatenate([q_v[...]] * (KS // DH), axis=1)
        for c in range(QS):
            p = jnp.exp(s_v[c] * scale - m)
            p_v[2 * c] = p[:, :VS]
            p_v[2 * c + 1] = p[:, VS:]
            for u in range(0, KS, DH):
                tot = tot + p[:, u:u + DH]
        l_v[...] = tot
        return carry

    jax.lax.fori_loop(0, NH, head, 0)

    def proj(ro, n, part):
        coef = jnp.concatenate([c_v[pl.ds(_mul(ro, 16), n), :]] * (D // DH), axis=1)
        prod = w_v[pl.ds(_mul(ro, 16), n), :].astype(F32) * coef
        return part + prod.reshape(n // 8, 8, D).sum(axis=0)

    def proj_piece(n, part):
        wo_piece(n).wait()
        return proj(wo_row(n), WR, part)

    def w_rows(ro):
        return w_v[pl.ds(_mul(ro, 16), FC), :]

    def start_quarter(u):
        n = N_FILL + 2 * NF + (u >> 2)
        wo_rows(wo_row(n) + (u & 3) * (WR // 4), WR // 4, n).start(priority=SHORT)

    def ffn(j, carry):
        hid, y, o, part = carry
        f0 = jnp.minimum(j * FC, F - FC)
        wo_piece(N_FILL + 2 * j).start(priority=SHORT)
        for g, a in enumerate(F_GROUPS[:-1]):
            @pl.when(j == a)
            def _():
                for c in long_f[g]:
                    c.wait()
        for u in range(FP):
            wo_piece(FP * j + u).wait()
        pl.delay(1)
        gt = jax.lax.dot_general(xn8, w_rows(GO + f0), _NT, preferred_element_type=F32)
        up = jax.lax.dot_general(xn8, w_rows(UO + f0), _NT, preferred_element_type=F32)
        o = jnp.where(j < 2 * QS, pv(1, NH - 1, jnp.minimum(j, 2 * QS - 1), 1, o), o)
        t = jnp.dot(hid.astype(BF16), w_rows(DO + jnp.maximum(j - 1, 0) * FC), preferred_element_type=F32)
        wo_piece(N_FILL + 2 * j + 1).start(priority=SHORT)
        start_quarter(j)
        for u in range(FP):
            part = proj(wo_row(FP * j + u), WR, part)
        col = f0 + jax.lax.broadcasted_iota(jnp.int32, (8, FC), 1)
        hid = jnp.where(col >= j * FC, jax.nn.silu(gt) * up, 0.0)
        y = jnp.where(j > 0, y + t, y)
        pl.delay(1)
        return hid, y, o, part

    zero = jnp.zeros((8, D), F32)
    hid, y, o, part = jax.lax.fori_loop(
        0, NF, ffn, (jnp.zeros((8, FC), F32), zero, jnp.zeros((8, DH), F32), zero))
    n1 = N_FILL + 2 * NF + 3
    wo_piece(n1).start(priority=SHORT)
    start_quarter(NF)
    q_v[...] = o / jnp.sum(l_v[...], axis=-1, keepdims=True)
    y = y + jnp.dot(hid.astype(BF16), w_rows(DO + F - FC), preferred_element_type=F32)
    pl.delay(1)
    wo_piece(n1 + 1).start(priority=SHORT)
    column(NH - 1, q_v[...])
    gate = jax.nn.silu(xn + (xn * 0.0 + y * jax.nn.sigmoid(r)))
    pl.delay(1)

    lag = 2 * (n1 + 2) - FP * NF

    def slots(lo, hi, prios, pause, part):
        def slot(n, part):
            for e, prio in enumerate(prios):
                wo_rows(wo_row(n) + e * (WR // 2), WR // 2, n).start(priority=prio)
                part = proj_piece(2 * n - lag + e, part)
                pl.delay(pause)
            return part
        return jax.lax.fori_loop(lo, hi, slot, part)

    n2, n3 = N_PACED - N_SPLIT, N_PACED - 1
    part = slots(n1 + 2, n2, (SHORT, SHORT), T_WO, part)
    part = slots(n2, n3, (SHORT, LONG), T_SPLIT, part)
    tail = ((wo_row(n3), LAST, n3), (wo_row(n3) + LAST, WR - LAST, 64))
    for rows, prio in zip(tail, (SHORT, LONG)):
        wo_rows(*rows).start(priority=prio)
        pl.delay(1)
    for n in list(range(2 * n3 - lag, n2)) + list(range(N_PACED, 63)):
        part = proj_piece(n, part)
    for a, n in wrap:
        wo_rows(a, n, 63).wait()
    for a, n in wrap:
        part = proj(a, n, part)
    for n in range(n2, n3):
        part = proj_piece(n, part)
    for a, n, s in tail[::-1]:
        wo_rows(a, n, s).wait()
        part = proj(a, n, part)
    s_out = jnp.sum(part, axis=0, keepdims=True)

    res = jnp.broadcast_to(x, (8, D)) + jnp.broadcast_to(s_out, (8, D)) * gate
    out_ref[0] = res.astype(out_ref.dtype)[0:1]


@jax.jit
def pallas_recurrent_scan__sliding_block_cached__moe_arch_mod__decode_kernel(
    A_x: jax.Array,
    A_k_cache: jax.Array,
    A_v_cache: jax.Array,
    A_wq: jax.Array,
    A_wo: jax.Array,
    B_x: jax.Array,
    B_w_r: jax.Array,
    B_w_gate: jax.Array,
    B_w_up: jax.Array,
    B_w_down: jax.Array,
):
    del B_x
    hbm = pl.BlockSpec(memory_space=pltpu.HBM)
    dma = pltpu.SemaphoreType.DMA
    return pl.pallas_call(
        _kernel,
        out_shape=jax.ShapeDtypeStruct((1, 1, D), BF16),
        in_specs=[hbm] * 9,
        out_specs=pl.BlockSpec(memory_space=pltpu.VMEM),
        scratch_shapes=[
            pltpu.VMEM((1, 1, D), BF16),
            pltpu.VMEM((D,), BF16),
            pltpu.VMEM((D, NH * DH), BF16),
            pltpu.VMEM((2, NH, W, DH), BF16),
            pltpu.VMEM((NH * DH + 3 * F, D), BF16),
            pltpu.VMEM((8, DH), F32),
            pltpu.VMEM((QS, 8, KS), F32),
            pltpu.VMEM((2 * QS, 8, VS), F32),
            pltpu.VMEM((8, DH), F32),
            pltpu.VMEM((NH * DH, DH), F32),
            dma((2,)), dma, dma((len(F_GROUPS) - 1,)), dma((2, 2)), dma((len(K_GROUPS) - 1,)), dma((65,)),
        ],
        compiler_params=pltpu.CompilerParams(
            vmem_limit_bytes=100 * 1024 * 1024,
            disable_semaphore_checks=True,
            disable_bounds_checks=True,
        ),
    )(A_x, A_k_cache, A_v_cache, A_wq, A_wo, B_w_r, B_w_gate.T, B_w_up.T, B_w_down)
```

```python
import jax
import jax.numpy as jnp
import jax.experimental.pallas as pl
import jax.experimental.pallas.tpu as pltpu

D = 512
NH = 32
DH = 128
SK = 32768
W = min(4096, max(256, SK // 4))
F = 1376

KV0 = (128, 64)
WQ0 = 2048
WO0 = 32

PR = 256
NA = W // PR - 1
ER = PR // 8
NP = (12, NA)
K_GROUPS = (0, 2, 6, 12, 18, 25, 32)
WQ_LONG = 4
WR = 64
QS = 4
KS = W // QS
VS = KS // 2
FC = 128
NF = -(-F // FC)
F_GROUPS = (0, 7, 10, NF)
N_FILL = 20
N_PACED = 56
N_SPLIT = 5
LAST = 16
FP = 3
GO, UO, DO = NH * DH, NH * DH + F, NH * DH + 2 * F

T_KV, T_WQ, T_EDGE, T_FIRST, T_NORM = (44, 45), 46, 22, 100, (35, 1, 15)
T_Q, T_ATT, T_MAX, T_EXP, T_WO, T_SPLIT = 10, 1, 10, 46, 24, 14

BF16 = jnp.bfloat16
F32 = jnp.float32
_NT = (((1,), (1,)), ((), ()))
LONG, SHORT = 1, 0


def _mul(a, m):
    return a if isinstance(a, int) else pl.multiple_of(a, m)


def _kernel(x_h, k_h, v_h, wq_h, wo_h, wr_h, wg_h, wu_h, wd_h, out_ref,
            x_v, wr_v, wq_v, kv_v, w_v, q_v, s_v, p_v, l_v, c_v, s_x, s_wq, s_f, s_kv, s_k, s_wo):
    kv_h = (k_h, v_h)

    def start_rows(t, h, ro, n):
        pltpu.make_async_copy(kv_h[t].at[0, h, pl.ds(_mul(SK - W + ro, 16), n), :],
                              kv_v.at[t, h, pl.ds(_mul(ro, 16), n), :],
                              s_kv.at[t, (h >> 1) & 1]).start(priority=SHORT)

    def start_piece(t, u, c, idle=False):
        n = (u & 1) * NP[t] + c - (NA - NP[t])
        j = n >> 1
        h, ro = (u & ~1) + (n & 1), KV0[t] + ((j >> 1) + (j & 1) * ((NP[t] + 1) // 2)) * PR
        if idle:
            for e in range(2):
                start_rows(t, h, ro + e * PR // 2, PR // 2)
                pl.delay(T_KV[e])
        else:
            start_rows(t, h, ro, PR)

    def start_edge(t, h, e, n):
        start_rows(t, h, (KV0[t] + NA * PR + e * ER) & (W - 1), n * ER)

    def wait_pair(t, p):
        k0, k1 = KV0[t] + NP[t] * PR, KV0[t] + NA * PR
        for a, b in ((0, k0), (k1, W)) if k1 > k0 else ((0, W),):
            rows = kv_v.at[t, pl.ds(2 * p, 2), pl.ds(a, b - a), :]
            pltpu.make_async_copy(rows, rows, s_kv.at[t, p & 1]).wait()

    def wo_rows(ro, n, s):
        return pltpu.make_async_copy(wo_h.at[pl.ds(_mul(ro, 16), n), :], w_v.at[pl.ds(_mul(ro, 16), n), :],
                                     s_wo.at[s])

    def wo_row(n):
        return (n & 7) * 8 * WR + WO0 + (n >> 3) * WR

    def wo_piece(n):
        return wo_rows(wo_row(n), WR, n)

    def start_wq(n, pause=0, prio=SHORT):
        g = (n >> 3) + (n & 7) * 8
        for r, c0, c1 in ((g, WQ0, NH * DH), ((g + 1) & 63, 0, WQ0)):
            if c1 > c0:
                idx = (pl.ds(_mul(r * 8, 8), 8), pl.ds(c0, c1 - c0))
                pltpu.make_async_copy(wq_h.at[idx], wq_v.at[idx], s_wq).start(priority=prio)
            if pause and c1 == NH * DH:
                pl.delay(pause)

    def start_long(copies):
        for c in copies:
            c.start(priority=LONG)
            pl.delay(1)

    copy_x = pltpu.make_async_copy(x_h, x_v, s_x.at[0])
    copy_wr = pltpu.make_async_copy(wr_h, wr_v, s_x.at[1])
    long_k = [[pltpu.make_async_copy(k_h.at[0, pl.ds(a, b - a), pl.ds(SK - W + KV0[0] + j * PR, PR), :],
                                     kv_v.at[0, pl.ds(a, b - a), pl.ds(KV0[0] + j * PR, PR), :], s_k.at[g])
               for j in range(NP[0], NA)]
              for g, (a, b) in enumerate(zip(K_GROUPS, K_GROUPS[1:]))]
    long_f = [[pltpu.make_async_copy(src.at[pl.ds(a * FC, min(b * FC, F) - a * FC), :],
                                     w_v.at[pl.ds(o + a * FC, min(b * FC, F) - a * FC), :], s_f.at[g])
               for src, o in ((wg_h, GO), (wu_h, UO), (wd_h, DO))]
              for g, (a, b) in enumerate(zip(F_GROUPS, F_GROUPS[1:]))]
    wrap = [(a, n) for a, n in ((wo_row(63), WR - WO0), (0, WO0)) if n]

    def wq_slot(n, carry):
        start_wq(n, T_WQ)
        pl.delay(T_WQ)
        return carry

    start_long(long_k[0])
    start_wq(0)
    copy_x.start(priority=SHORT)
    copy_wr.start(priority=SHORT)
    pl.delay(T_FIRST)
    jax.lax.fori_loop(1, 6, wq_slot, 0)

    start_wq(6, T_WQ)
    copy_x.wait()
    copy_wr.wait()
    x = x_v[0].astype(F32)
    xc = x - jnp.mean(x, axis=-1, keepdims=True)
    pl.delay(T_NORM[0])
    start_wq(7, T_WQ)
    var = jnp.mean(jnp.square(xc), axis=-1, keepdims=True)
    xn_b = (xc / jnp.sqrt(var + 1e-5)).astype(BF16)
    xn = xn_b.astype(F32)
    xn8 = jnp.broadcast_to(xn_b, (8, D))
    pl.delay(T_NORM[1])
    start_wq(8, T_WQ)
    r = jnp.sum(xn * wr_v[...].reshape(1, D).astype(F32), axis=-1, keepdims=True)
    p_v[...] = jnp.zeros(p_v.shape, F32)
    l_v[...] = jnp.ones(l_v.shape, F32)
    pl.delay(T_NORM[2])

    for n in range(WQ_LONG):
        start_wq(9 + n, prio=LONG)
    pl.delay(1)
    start_long(sum(long_k[1:], []))
    jax.lax.fori_loop(9 + WQ_LONG, 64 - 3 * NP[0], wq_slot, 0)
    ahead = ((0, 0), (0, 1), (1, 0))
    for t, h in ahead:
        for e in range(0, 8, 2):
            start_edge(t, h, e, 2)
            pl.delay(T_EDGE)
    for c in range(NA - NP[0]):
        start_piece(1, 0, c, idle=True)

    def lead(c, carry):
        for u, (t, b) in enumerate(ahead):
            wq_slot(64 - 3 * (NA - c) + u, 0)
            start_piece(t, b, c, idle=True)
        return carry

    jax.lax.fori_loop(NA - NP[0], NA, lead, 0)

    scale = DH ** -0.5

    def pv(t, h, c, n, o):
        p = jnp.concatenate([p_v[c + u] for u in range(n)], axis=1).astype(BF16)
        return o + jnp.dot(p, kv_v[t, h, pl.ds(_mul(c * VS, VS), n * VS), :], preferred_element_type=F32)

    def column(h, o):
        o = jnp.concatenate([o.astype(BF16).astype(F32)] * (DH // 8), axis=0)
        eye = (jax.lax.broadcasted_iota(jnp.int32, (DH, DH), 0)
               == jax.lax.broadcasted_iota(jnp.int32, (DH, DH), 1))
        col = jnp.sum(jnp.where(eye, o, 0.0), axis=-1, keepdims=True)
        c_v[pl.ds(_mul(h * DH, DH), DH), :] = jnp.broadcast_to(col, (DH, DH))

    def head(i, carry):
        def issue(t, c, n, edge=None):
            @pl.when(i + 2 - t < NH)
            def _():
                start_piece(t, i + 2 - t, c)
                if edge is not None:
                    start_edge(t, i + 2 - t, *edge)

            @pl.when(i + 2 - t >= NH)
            def _():
                wo_piece(n).start(priority=SHORT)

        def fill(u):
            return jnp.where(i == NH - 2, u, 7 + 2 * u)

        def idle(c, carry):
            @pl.when(jnp.logical_and(i + 2 < NH, c >= NA - NP[0]))
            def _():
                start_piece(0, i + 2, c, idle=True)
            start_piece(1, i + 1, c, idle=True)
            return carry

        c0 = NA - QS - 3
        jax.lax.fori_loop(0, jnp.where(i + 1 < NH, c0, 0), idle, 0)
        for g, a in enumerate(K_GROUPS[:-1]):
            @pl.when(i == a)
            def _():
                for c in long_k[g]:
                    c.wait()
                if g == 0:
                    pltpu.make_async_copy(wq_v, wq_v, s_wq).wait()
                if g == 4:
                    start_long(sum(long_f, []) + [wo_piece(n) for n in range(N_PACED, 63)]
                               + [wo_rows(a_, n, 63) for a_, n in wrap])
        for t in range(2):
            @pl.when((i & 1) == t)
            def _():
                wait_pair(t, i >> 1)
        hp = jnp.maximum(i - 1, 0)
        tp = jnp.minimum(i, 1)

        issue(0, c0, fill(0))
        pl.delay(T_Q)
        l_v[...] = jnp.broadcast_to(jnp.sum(l_v[...], axis=-1, keepdims=True), (8, DH))
        q_v[...] = jnp.dot(xn8, wq_v[:, pl.ds(pl.multiple_of(i * DH, DH), DH)], preferred_element_type=F32)
        o = pv(tp, hp, 4, 2, jnp.zeros((8, DH), F32))
        issue(1, c0, 8)
        pl.delay(1)

        def att(c, o):
            issue(0, c0 + 1 + c, fill(1 + c), (c, 1))
            pl.delay(T_ATT)
            s = jax.lax.dot_general(q_v[...].astype(BF16), kv_v[0, i, pl.ds(pl.multiple_of(c * KS, KS), KS), :],
                                    _NT, preferred_element_type=F32)
            o = pv(tp, hp, c, 1, o)
            issue(1, c0 + 1 + c, 10 + 2 * c, (c, 1))
            s_v[c] = s
            pl.delay(1)
            return o

        o = jax.lax.fori_loop(0, QS, att, o)

        issue(0, NA - 2, fill(5))
        mx = None
        for c in range(QS):
            s = s_v[c] * scale
            for u in range(0, KS, DH):
                mx = s[:, u:u + DH] if mx is None else jnp.maximum(mx, s[:, u:u + DH])
        pl.delay(T_MAX)

        @pl.when(i + 2 < NH)
        def _():
            start_edge(0, i + 2, 4, 2)
        pl.delay(1)
        q_v[...] = jnp.broadcast_to(jnp.max(mx, axis=-1, keepdims=True), (8, DH))
        o = pv(tp, hp, 6, 2, o)
        issue(1, NA - 2, 18, (4, 2))
        pl.delay(1)

        issue(0, NA - 1, fill(6), (6, 2))
        column(hp, o / l_v[...])
        pl.delay(1)

        @pl.when(i + 1 < NH)
        def _():
            start_piece(1, i + 1, NA - 1)
            start_edge(1, i + 1, 6, 2)
            pl.delay(T_EXP)
        tot = jnp.zeros((8, DH), F32)
        m = jnp.concatenate([q_v[...]] * (KS // DH), axis=1)
        for c in range(QS):
            p = jnp.exp(s_v[c] * scale - m)
            p_v[2 * c] = p[:, :VS]
            p_v[2 * c + 1] = p[:, VS:]
            for u in range(0, KS, DH):
                tot = tot + p[:, u:u + DH]
        l_v[...] = tot
        return carry

    jax.lax.fori_loop(0, NH, head, 0)

    def proj(ro, n, part):
        coef = jnp.concatenate([c_v[pl.ds(_mul(ro, 16), n), :]] * (D // DH), axis=1)
        prod = w_v[pl.ds(_mul(ro, 16), n), :].astype(F32) * coef
        return part + prod.reshape(n // 8, 8, D).sum(axis=0)

    def proj_piece(n, part):
        wo_piece(n).wait()
        return proj(wo_row(n), WR, part)

    def w_rows(ro):
        return w_v[pl.ds(_mul(ro, 16), FC), :]

    def start_quarter(u):
        n = N_FILL + 2 * NF + (u >> 2)
        wo_rows(wo_row(n) + (u & 3) * (WR // 4), WR // 4, n).start(priority=SHORT)

    def ffn(j, carry):
        hid, y, o, part = carry
        f0 = jnp.minimum(j * FC, F - FC)
        wo_piece(N_FILL + 2 * j).start(priority=SHORT)
        for g, a in enumerate(F_GROUPS[:-1]):
            @pl.when(j == a)
            def _():
                for c in long_f[g]:
                    c.wait()
        for u in range(FP):
            wo_piece(FP * j + u).wait()
        pl.delay(1)
        gt = jax.lax.dot_general(xn8, w_rows(GO + f0), _NT, preferred_element_type=F32)
        up = jax.lax.dot_general(xn8, w_rows(UO + f0), _NT, preferred_element_type=F32)
        o = jnp.where(j < 2 * QS, pv(1, NH - 1, jnp.minimum(j, 2 * QS - 1), 1, o), o)
        t = jnp.dot(hid.astype(BF16), w_rows(DO + jnp.maximum(j - 1, 0) * FC), preferred_element_type=F32)
        wo_piece(N_FILL + 2 * j + 1).start(priority=SHORT)
        start_quarter(j)
        for u in range(FP):
            part = proj(wo_row(FP * j + u), WR, part)
        col = f0 + jax.lax.broadcasted_iota(jnp.int32, (8, FC), 1)
        hid = jnp.where(col >= j * FC, jax.nn.silu(gt) * up, 0.0)
        y = jnp.where(j > 0, y + t, y)
        pl.delay(1)
        return hid, y, o, part

    zero = jnp.zeros((8, D), F32)
    hid, y, o, part = jax.lax.fori_loop(
        0, NF, ffn, (jnp.zeros((8, FC), F32), zero, jnp.zeros((8, DH), F32), zero))
    n1 = N_FILL + 2 * NF + 3
    wo_piece(n1).start(priority=SHORT)
    start_quarter(NF)
    q_v[...] = o / jnp.sum(l_v[...], axis=-1, keepdims=True)
    y = y + jnp.dot(hid.astype(BF16), w_rows(DO + F - FC), preferred_element_type=F32)
    pl.delay(1)
    wo_piece(n1 + 1).start(priority=SHORT)
    column(NH - 1, q_v[...])
    gate = jax.nn.silu(xn + (xn * 0.0 + y * jax.nn.sigmoid(r)))
    pl.delay(1)

    lag = 2 * (n1 + 2) - FP * NF

    def slots(lo, hi, prios, pause, part):
        def slot(n, part):
            for e, prio in enumerate(prios):
                wo_rows(wo_row(n) + e * (WR // 2), WR // 2, n).start(priority=prio)
                part = proj_piece(2 * n - lag + e, part)
                pl.delay(pause)
            return part
        return jax.lax.fori_loop(lo, hi, slot, part)

    n2, n3 = N_PACED - N_SPLIT, N_PACED - 1
    part = slots(n1 + 2, n2, (SHORT, SHORT), T_WO, part)
    part = slots(n2, n3, (SHORT, LONG), T_SPLIT, part)
    tail = ((wo_row(n3), LAST, n3), (wo_row(n3) + LAST, WR - LAST, 64))
    for rows, prio in zip(tail, (SHORT, LONG)):
        wo_rows(*rows).start(priority=prio)
        pl.delay(1)
    for n in list(range(2 * n3 - lag, n2)) + list(range(N_PACED, 63)):
        part = proj_piece(n, part)
    for a, n in wrap:
        wo_rows(a, n, 63).wait()
    for a, n in wrap:
        part = proj(a, n, part)
    for n in range(n2, n3):
        part = proj_piece(n, part)
    for a, n, s in tail[::-1]:
        wo_rows(a, n, s).wait()
        part = proj(a, n, part)
    s_out = jnp.sum(part, axis=0, keepdims=True)

    res = jnp.broadcast_to(x, (8, D)) + jnp.broadcast_to(s_out, (8, D)) * gate
    out_ref[0] = res.astype(out_ref.dtype)[0:1]


@jax.jit
def pallas_recurrent_scan__sliding_block_cached__moe_arch_mod__decode_kernel(
    A_x: jax.Array,
    A_k_cache: jax.Array,
    A_v_cache: jax.Array,
    A_wq: jax.Array,
    A_wo: jax.Array,
    B_x: jax.Array,
    B_w_r: jax.Array,
    B_w_gate: jax.Array,
    B_w_up: jax.Array,
    B_w_down: jax.Array,
):
    del B_x
    hbm = pl.BlockSpec(memory_space=pltpu.HBM)
    dma = pltpu.SemaphoreType.DMA
    return pl.pallas_call(
        _kernel,
        out_shape=jax.ShapeDtypeStruct((1, 1, D), BF16),
        in_specs=[hbm] * 9,
        out_specs=pl.BlockSpec(memory_space=pltpu.VMEM),
        scratch_shapes=[
            pltpu.VMEM((1, 1, D), BF16),
            pltpu.VMEM((D,), BF16),
            pltpu.VMEM((D, NH * DH), BF16),
            pltpu.VMEM((2, NH, W, DH), BF16),
            pltpu.VMEM((NH * DH + 3 * F, D), BF16),
            pltpu.VMEM((8, DH), F32),
            pltpu.VMEM((QS, 8, KS), F32),
            pltpu.VMEM((2 * QS, 8, VS), F32),
            pltpu.VMEM((8, DH), F32),
            pltpu.VMEM((NH * DH, DH), F32),
            dma((2,)), dma, dma((len(F_GROUPS) - 1,)), dma((2, 2)), dma((len(K_GROUPS) - 1,)), dma((65,)),
        ],
        compiler_params=pltpu.CompilerParams(
            vmem_limit_bytes=100 * 1024 * 1024,
            disable_semaphore_checks=True,
            disable_bounds_checks=True,
        ),
    )(A_x, A_k_cache, A_v_cache, A_wq, A_wo, B_w_r, B_w_gate.T, B_w_up.T, B_w_down)
```

```python
import jax
import jax.numpy as jnp
import jax.experimental.pallas as pl
import jax.experimental.pallas.tpu as pltpu

D = 512
NH = 32
DH = 128
SK = 32768
W = min(4096, max(256, SK // 4))
F = 1376

KV0 = (128, 64)
WQ0 = 2048
WO0 = 32

PR = 256
NA = W // PR - 1
ER = PR // 8
NP = (12, NA)
K_GROUPS = (0, 2, 6, 12, 18, 25, 32)
WQ_LONG = 4
WR = 64
QS = 4
KS = W // QS
VS = KS // 2
FC = 128
NF = -(-F // FC)
F_GROUPS = (0, 7, 10, NF)
N_FILL = 20
N_PACED = 56
N_SPLIT = 5
LAST = 16
FP = 3
GO, UO, DO = NH * DH, NH * DH + F, NH * DH + 2 * F

T_KV, T_WQ, T_EDGE, T_FIRST, T_NORM = (44, 45), 46, 22, 100, (35, 1, 15)
T_Q, T_ATT, T_MAX, T_EXP, T_WO, T_SPLIT = 10, 1, 10, 46, 24, 14

BF16 = jnp.bfloat16
F32 = jnp.float32
_NT = (((1,), (1,)), ((), ()))
LONG, SHORT = 1, 0


def _mul(a, m):
    return a if isinstance(a, int) else pl.multiple_of(a, m)


def _kernel(x_h, k_h, v_h, wq_h, wo_h, wr_h, wg_h, wu_h, wd_h, out_ref,
            x_v, wr_v, wq_v, kv_v, w_v, q_v, s_v, p_v, l_v, c_v, s_x, s_wq, s_f, s_kv, s_k, s_wo):
    kv_h = (k_h, v_h)

    def start_rows(t, h, ro, n, s):
        pltpu.make_async_copy(kv_h[t].at[0, h, pl.ds(_mul(SK - W + ro, 16), n), :],
                              kv_v.at[t, h, pl.ds(_mul(ro, 16), n), :],
                              s_kv.at[s, (h >> 1) & 1]).start(priority=SHORT)

    def start_piece(t, u, c, idle=False):
        n = (u & 1) * NP[t] + c - (NA - NP[t])
        j = n >> 1
        h, ro = (u & ~1) + (n & 1), KV0[t] + ((j >> 1) + (j & 1) * ((NP[t] + 1) // 2)) * PR
        if idle:
            for e in range(2):
                start_rows(t, h, ro + e * PR // 2, PR // 2, t)
                pl.delay(T_KV[e])
        else:
            start_rows(t, h, ro, PR, t)

    def start_edge(t, h, e, n):
        ro = KV0[t] + NA * PR + e * ER
        start_rows(t, h, ro & (W - 1), n * ER, 1 if t else 2 - 2 * (ro >> (W.bit_length() - 1)))

    def wait_pair(t, p):
        k0, k1 = KV0[0] + NP[0] * PR, KV0[0] + NA * PR
        for a, b, s in ((0, W, 1),) if t else ((0, k0, 0), (k1, W, 2)):
            rows = kv_v.at[t, pl.ds(2 * p, 2), pl.ds(a, b - a), :]
            pltpu.make_async_copy(rows, rows, s_kv.at[s, p & 1]).wait()

    def wo_rows(ro, n, s):
        return pltpu.make_async_copy(wo_h.at[pl.ds(_mul(ro, 16), n), :], w_v.at[pl.ds(_mul(ro, 16), n), :],
                                     s_wo.at[s])

    def wo_row(n):
        return (n & 7) * 8 * WR + WO0 + (n >> 3) * WR

    def wo_piece(n):
        return wo_rows(wo_row(n), WR, n)

    def start_wq(n, pause=0, prio=SHORT):
        g = (n >> 3) + (n & 7) * 8
        for r, c0, c1 in ((g, WQ0, NH * DH), ((g + 1) & 63, 0, WQ0)):
            if c1 > c0:
                idx = (pl.ds(_mul(r * 8, 8), 8), pl.ds(c0, c1 - c0))
                pltpu.make_async_copy(wq_h.at[idx], wq_v.at[idx], s_wq).start(priority=prio)
            if pause and c1 == NH * DH:
                pl.delay(pause)

    def start_long(copies):
        for c in copies:
            c.start(priority=LONG)
            pl.delay(1)

    copy_x = pltpu.make_async_copy(x_h, x_v, s_x.at[0])
    copy_wr = pltpu.make_async_copy(wr_h, wr_v, s_x.at[1])
    long_k = [[pltpu.make_async_copy(k_h.at[0, pl.ds(a, b - a), pl.ds(SK - W + KV0[0] + j * PR, PR), :],
                                     kv_v.at[0, pl.ds(a, b - a), pl.ds(KV0[0] + j * PR, PR), :], s_k.at[g])
               for j in range(NP[0], NA)]
              for g, (a, b) in enumerate(zip(K_GROUPS, K_GROUPS[1:]))]
    long_f = [[pltpu.make_async_copy(src.at[pl.ds(a * FC, min(b * FC, F) - a * FC), :],
                                     w_v.at[pl.ds(o + a * FC, min(b * FC, F) - a * FC), :], s_f.at[g])
               for src, o in ((wg_h, GO), (wu_h, UO), (wd_h, DO))]
              for g, (a, b) in enumerate(zip(F_GROUPS, F_GROUPS[1:]))]
    wrap = [(a, n) for a, n in ((wo_row(63), WR - WO0), (0, WO0)) if n]

    def wq_slot(n, carry):
        start_wq(n, T_WQ)
        pl.delay(T_WQ)
        return carry

    start_long(long_k[0])
    start_wq(0)
    copy_x.start(priority=SHORT)
    copy_wr.start(priority=SHORT)
    pl.delay(T_FIRST)
    jax.lax.fori_loop(1, 6, wq_slot, 0)

    start_wq(6, T_WQ)
    copy_x.wait()
    copy_wr.wait()
    x = x_v[0].astype(F32)
    xc = x - jnp.mean(x, axis=-1, keepdims=True)
    pl.delay(T_NORM[0])
    start_wq(7, T_WQ)
    var = jnp.mean(jnp.square(xc), axis=-1, keepdims=True)
    xn_b = (xc / jnp.sqrt(var + 1e-5)).astype(BF16)
    xn = xn_b.astype(F32)
    xn8 = jnp.broadcast_to(xn_b, (8, D))
    pl.delay(T_NORM[1])
    start_wq(8, T_WQ)
    r = jnp.sum(xn * wr_v[...].reshape(1, D).astype(F32), axis=-1, keepdims=True)
    p_v[...] = jnp.zeros(p_v.shape, F32)
    l_v[...] = jnp.ones(l_v.shape, F32)
    pl.delay(T_NORM[2])

    for n in range(WQ_LONG):
        start_wq(9 + n, prio=LONG)
    pl.delay(1)
    start_long(sum(long_k[1:], []))
    jax.lax.fori_loop(9 + WQ_LONG, 64 - 3 * NP[0], wq_slot, 0)
    ahead = ((0, 0), (0, 1), (1, 0))
    for t, h in ahead:
        for e in range(0, 8, 2):
            start_edge(t, h, e, 2)
            pl.delay(T_EDGE)
    for c in range(NA - NP[0]):
        start_piece(1, 0, c, idle=True)

    def lead(c, carry):
        for u, (t, b) in enumerate(ahead):
            wq_slot(64 - 3 * (NA - c) + u, 0)
            start_piece(t, b, c, idle=True)
        return carry

    jax.lax.fori_loop(NA - NP[0], NA, lead, 0)

    scale = DH ** -0.5

    def pv(t, h, c, n, o):
        p = jnp.concatenate([p_v[c + u] for u in range(n)], axis=1).astype(BF16)
        return o + jnp.dot(p, kv_v[t, h, pl.ds(_mul(c * VS, VS), n * VS), :], preferred_element_type=F32)

    def column(h, o):
        o = jnp.concatenate([o.astype(BF16).astype(F32)] * (DH // 8), axis=0)
        eye = (jax.lax.broadcasted_iota(jnp.int32, (DH, DH), 0)
               == jax.lax.broadcasted_iota(jnp.int32, (DH, DH), 1))
        col = jnp.sum(jnp.where(eye, o, 0.0), axis=-1, keepdims=True)
        c_v[pl.ds(_mul(h * DH, DH), DH), :] = jnp.broadcast_to(col, (DH, DH))

    def head(i, carry):
        def issue(t, c, n, edge=None):
            @pl.when(i + 2 - t < NH)
            def _():
                start_piece(t, i + 2 - t, c)
                if edge is not None:
                    start_edge(t, i + 2 - t, *edge)

            @pl.when(i + 2 - t >= NH)
            def _():
                wo_piece(n).start(priority=SHORT)

        def fill(u):
            return jnp.where(i == NH - 2, u, 7 + 2 * u)

        def idle(c, carry):
            @pl.when(jnp.logical_and(i + 2 < NH, c >= NA - NP[0]))
            def _():
                start_piece(0, i + 2, c, idle=True)
            start_piece(1, i + 1, c, idle=True)
            return carry

        c0 = NA - QS - 3
        jax.lax.fori_loop(0, jnp.where(i + 1 < NH, c0, 0), idle, 0)
        for g, a in enumerate(K_GROUPS[:-1]):
            @pl.when(i == a)
            def _():
                for c in long_k[g]:
                    c.wait()
                if g == 0:
                    pltpu.make_async_copy(wq_v, wq_v, s_wq).wait()
                if g == 4:
                    start_long(sum(long_f, []) + [wo_piece(n) for n in range(N_PACED, 63)]
                               + [wo_rows(a_, n, 63) for a_, n in wrap])
        for t in range(2):
            @pl.when((i & 1) == t)
            def _():
                wait_pair(t, i >> 1)
        hp = jnp.maximum(i - 1, 0)
        tp = jnp.minimum(i, 1)

        issue(0, c0, fill(0))
        pl.delay(T_Q)
        l_v[...] = jnp.broadcast_to(jnp.sum(l_v[...], axis=-1, keepdims=True), (8, DH))
        q_v[...] = jnp.dot(xn8, wq_v[:, pl.ds(pl.multiple_of(i * DH, DH), DH)], preferred_element_type=F32)
        o = pv(tp, hp, 4, 2, jnp.zeros((8, DH), F32))
        issue(1, c0, 8)
        pl.delay(1)

        def att(c, o):
            issue(0, c0 + 1 + c, fill(1 + c), (c, 1))
            pl.delay(T_ATT)
            s = jax.lax.dot_general(q_v[...].astype(BF16), kv_v[0, i, pl.ds(pl.multiple_of(c * KS, KS), KS), :],
                                    _NT, preferred_element_type=F32)
            o = pv(tp, hp, c, 1, o)
            issue(1, c0 + 1 + c, 10 + 2 * c, (c, 1))
            s_v[c] = s
            pl.delay(1)
            return o

        o = jax.lax.fori_loop(0, QS, att, o)

        issue(0, NA - 2, fill(5))
        mx = None
        for c in range(QS):
            s = s_v[c] * scale
            for u in range(0, KS, DH):
                mx = s[:, u:u + DH] if mx is None else jnp.maximum(mx, s[:, u:u + DH])
        pl.delay(T_MAX)

        @pl.when(i + 2 < NH)
        def _():
            start_edge(0, i + 2, 4, 2)
        pl.delay(1)
        q_v[...] = jnp.broadcast_to(jnp.max(mx, axis=-1, keepdims=True), (8, DH))
        o = pv(tp, hp, 6, 2, o)
        issue(1, NA - 2, 18, (4, 2))
        pl.delay(1)

        issue(0, NA - 1, fill(6), (6, 2))
        column(hp, o / l_v[...])
        pl.delay(1)

        @pl.when(i + 1 < NH)
        def _():
            start_piece(1, i + 1, NA - 1)
            start_edge(1, i + 1, 6, 2)
            pl.delay(T_EXP)
        tot = jnp.zeros((8, DH), F32)
        m = jnp.concatenate([q_v[...]] * (KS // DH), axis=1)
        for c in range(QS):
            p = jnp.exp(s_v[c] * scale - m)
            p_v[2 * c] = p[:, :VS]
            p_v[2 * c + 1] = p[:, VS:]
            for u in range(0, KS, DH):
                tot = tot + p[:, u:u + DH]
        l_v[...] = tot
        return carry

    jax.lax.fori_loop(0, NH, head, 0)

    def proj(ro, n, part):
        coef = jnp.concatenate([c_v[pl.ds(_mul(ro, 16), n), :]] * (D // DH), axis=1)
        prod = w_v[pl.ds(_mul(ro, 16), n), :].astype(F32) * coef
        return part + prod.reshape(n // 8, 8, D).sum(axis=0)

    def proj_piece(n, part):
        wo_piece(n).wait()
        return proj(wo_row(n), WR, part)

    def w_rows(ro):
        return w_v[pl.ds(_mul(ro, 16), FC), :]

    def start_quarter(u):
        n = N_FILL + 2 * NF + (u >> 2)
        wo_rows(wo_row(n) + (u & 3) * (WR // 4), WR // 4, n).start(priority=SHORT)

    def ffn(j, carry):
        hid, y, o, part = carry
        f0 = jnp.minimum(j * FC, F - FC)
        wo_piece(N_FILL + 2 * j).start(priority=SHORT)
        for g, a in enumerate(F_GROUPS[:-1]):
            @pl.when(j == a)
            def _():
                for c in long_f[g]:
                    c.wait()
        for u in range(FP):
            wo_piece(FP * j + u).wait()
        pl.delay(1)
        gt = jax.lax.dot_general(xn8, w_rows(GO + f0), _NT, preferred_element_type=F32)
        up = jax.lax.dot_general(xn8, w_rows(UO + f0), _NT, preferred_element_type=F32)
        o = jnp.where(j < 2 * QS, pv(1, NH - 1, jnp.minimum(j, 2 * QS - 1), 1, o), o)
        t = jnp.dot(hid.astype(BF16), w_rows(DO + jnp.maximum(j - 1, 0) * FC), preferred_element_type=F32)
        wo_piece(N_FILL + 2 * j + 1).start(priority=SHORT)
        start_quarter(j)
        for u in range(FP):
            part = proj(wo_row(FP * j + u), WR, part)
        col = f0 + jax.lax.broadcasted_iota(jnp.int32, (8, FC), 1)
        hid = jnp.where(col >= j * FC, jax.nn.silu(gt) * up, 0.0)
        y = jnp.where(j > 0, y + t, y)
        pl.delay(1)
        return hid, y, o, part

    zero = jnp.zeros((8, D), F32)
    hid, y, o, part = jax.lax.fori_loop(
        0, NF, ffn, (jnp.zeros((8, FC), F32), zero, jnp.zeros((8, DH), F32), zero))
    n1 = N_FILL + 2 * NF + 3
    wo_piece(n1).start(priority=SHORT)
    start_quarter(NF)
    q_v[...] = o / jnp.sum(l_v[...], axis=-1, keepdims=True)
    y = y + jnp.dot(hid.astype(BF16), w_rows(DO + F - FC), preferred_element_type=F32)
    pl.delay(1)
    wo_piece(n1 + 1).start(priority=SHORT)
    column(NH - 1, q_v[...])
    gate = jax.nn.silu(xn + (xn * 0.0 + y * jax.nn.sigmoid(r)))
    pl.delay(1)

    lag = 2 * (n1 + 2) - FP * NF

    def slots(lo, hi, prios, pause, part):
        def slot(n, part):
            for e, prio in enumerate(prios):
                wo_rows(wo_row(n) + e * (WR // 2), WR // 2, n).start(priority=prio)
                part = proj_piece(2 * n - lag + e, part)
                pl.delay(pause)
            return part
        return jax.lax.fori_loop(lo, hi, slot, part)

    n2, n3 = N_PACED - N_SPLIT, N_PACED - 1
    part = slots(n1 + 2, n2, (SHORT, SHORT), T_WO, part)
    part = slots(n2, n3, (SHORT, LONG), T_SPLIT, part)
    tail = ((wo_row(n3), LAST, n3), (wo_row(n3) + LAST, WR - LAST, 64))
    for rows, prio in zip(tail, (SHORT, LONG)):
        wo_rows(*rows).start(priority=prio)
        pl.delay(1)
    for n in list(range(2 * n3 - lag, n2)) + list(range(N_PACED, 63)):
        part = proj_piece(n, part)
    for a, n in wrap:
        wo_rows(a, n, 63).wait()
    for a, n in wrap:
        part = proj(a, n, part)
    for n in range(n2, n3):
        part = proj_piece(n, part)
    for a, n, s in tail[::-1]:
        wo_rows(a, n, s).wait()
        part = proj(a, n, part)
    s_out = jnp.sum(part, axis=0, keepdims=True)

    res = jnp.broadcast_to(x, (8, D)) + jnp.broadcast_to(s_out, (8, D)) * gate
    out_ref[0] = res.astype(out_ref.dtype)[0:1]


@jax.jit
def pallas_recurrent_scan__sliding_block_cached__moe_arch_mod__decode_kernel(
    A_x: jax.Array,
    A_k_cache: jax.Array,
    A_v_cache: jax.Array,
    A_wq: jax.Array,
    A_wo: jax.Array,
    B_x: jax.Array,
    B_w_r: jax.Array,
    B_w_gate: jax.Array,
    B_w_up: jax.Array,
    B_w_down: jax.Array,
):
    del B_x
    hbm = pl.BlockSpec(memory_space=pltpu.HBM)
    dma = pltpu.SemaphoreType.DMA
    return pl.pallas_call(
        _kernel,
        out_shape=jax.ShapeDtypeStruct((1, 1, D), BF16),
        in_specs=[hbm] * 9,
        out_specs=pl.BlockSpec(memory_space=pltpu.VMEM),
        scratch_shapes=[
            pltpu.VMEM((1, 1, D), BF16),
            pltpu.VMEM((D,), BF16),
            pltpu.VMEM((D, NH * DH), BF16),
            pltpu.VMEM((2, NH, W, DH), BF16),
            pltpu.VMEM((NH * DH + 3 * F, D), BF16),
            pltpu.VMEM((8, DH), F32),
            pltpu.VMEM((QS, 8, KS), F32),
            pltpu.VMEM((2 * QS, 8, VS), F32),
            pltpu.VMEM((8, DH), F32),
            pltpu.VMEM((NH * DH, DH), F32),
            dma((2,)), dma, dma((len(F_GROUPS) - 1,)), dma((3, 2)), dma((len(K_GROUPS) - 1,)), dma((65,)),
        ],
        compiler_params=pltpu.CompilerParams(
            vmem_limit_bytes=100 * 1024 * 1024,
            disable_semaphore_checks=True,
            disable_bounds_checks=True,
        ),
    )(A_x, A_k_cache, A_v_cache, A_wq, A_wo, B_w_r, B_w_gate.T, B_w_up.T, B_w_down)
```
